```python
import jax
import jax.numpy as jnp

def _softmax(x, axis=-1):
    return jax.nn.softmax(x, axis=axis)
def _gelu(x):
    return jax.nn.gelu(x, approximate=True)
def _silu(x):
    return jax.nn.silu(x)
def _sigmoid(x):
    return jax.nn.sigmoid(x)
def _layernorm(x, axis=-1, eps=1e-5):
    m = jnp.mean(x, axis=axis, keepdims=True)
    v = jnp.var(x, axis=axis, keepdims=True)
    return (x - m) / jnp.sqrt(v + eps)
def _scatter_add(tgt, idx, src, axis=0):
    return tgt.at[idx].add(src)
def _segment_sum(src, seg, n):
    return jax.ops.segment_sum(src, seg, n)
class _Rng:
    def __init__(self, key):
        self._k = key
    def _next(self):
        self._k, sub = jax.random.split(self._k)
        return sub
    def normal(self, shape):
        return jax.random.normal(self._next(), shape, dtype=jnp.bfloat16)
    def randint(self, lo, hi, shape):
        return jax.random.randint(self._next(), shape, lo, hi, dtype=jnp.int32)
    def uniform(self, shape, lo=0.0, hi=1.0):
        return jax.random.uniform(self._next(), shape, jnp.bfloat16, lo, hi)
    def permutation(self, n):
        return jax.random.permutation(self._next(), n)


kernel_name = 'parallel_sum__linear_attn_block__moe_arch_mod__prompt'

def setup_inputs():
    _rng = _Rng(jax.random.key(int.from_bytes(__import__("os").urandom(4), "little")))
    _w = (lambda a: (lambda t: t.astype(jnp.bfloat16) if jnp.issubdtype(t.dtype, jnp.floating) else t)(jnp.asarray(a)))
    def _A_setup():
        B, S, D = 1, 2048, 1024
        return {
            "x": _w((lambda *s: _rng.normal(s) * 0.05)(B, S, D)),
            "wqkv": _w((lambda *s: _rng.normal(s) * 0.05)(D, 3 * D)),
            "wo": _w((lambda *s: _rng.normal(s) * 0.05)(D, D)),
        }
    _A_in = _A_setup()

    def _B_setup():
        B, S, D, F, C = 1, 2048, 1024, 3584, 1
        return {
            "x": _w((lambda *s: _rng.normal(s) * 0.05)(B, S, D)),
            "w_r": _w((lambda *s: _rng.normal(s) * 0.05)(D)),
            "w_gate": _w((lambda *s: _rng.normal(s) * 0.05)(D, F)),
            "w_up": _w((lambda *s: _rng.normal(s) * 0.05)(D, F)),
            "w_down": _w((lambda *s: _rng.normal(s) * 0.05)(F, D)),
        }
    _B_in = _B_setup()

    return {
        "A_x": _A_in["x"],
        "A_wqkv": _A_in["wqkv"],
        "A_wo": _A_in["wo"],
        "B_x": _B_in["x"],
        "B_w_r": _B_in["w_r"],
        "B_w_gate": _B_in["w_gate"],
        "B_w_up": _B_in["w_up"],
        "B_w_down": _B_in["w_down"],
    }

def reference(A_x, A_wqkv, A_wo, B_x, B_w_r, B_w_gate, B_w_up, B_w_down):
    def _A_ref(x, wqkv, wo):
        B, S, D = x.shape
        H = 32; Dh = D // H
        qkv = (lambda x, *d: x.transpose(*d))((x @ wqkv).reshape(B, S, 3, H, Dh), 2, 0, 3, 1, 4)
        q, k, v = qkv[0], qkv[1], qkv[2]
        phi = lambda t: jnp.where(t > 0, t + 1, jnp.exp(t)) + 1e-6
        pq, pk = phi(q), phi(k)
        kv = jnp.einsum("bhsd,bhse->bhde", pk, v)
        z = jnp.einsum("bhsd->bhd", pk)
        num = jnp.einsum("bhqd,bhde->bhqe", pq, kv)
        den = jnp.einsum("bhqd,bhd->bhq", pq, z)[..., None] + 1e-6
        o = num / den
        return (lambda x, *d: x.transpose(*d))(o, 0, 2, 1, 3).reshape(B, S, D) @ wo

    def _B_ref(x, w_r, w_gate, w_up, w_down):
        B, S, D = x.shape
        C = 1
        r = x @ w_r
        idx = jnp.argsort(-r, axis=-1)[:, :C]
        idx_e = jnp.repeat(idx.reshape(B, C, 1), D, axis=2)
        x_sel = jnp.take_along_axis(x, idx_e, axis=1)
        g = _silu(x_sel @ w_gate)
        u = x_sel @ w_up
        y = (g * u) @ w_down
        r_sel = _sigmoid(jnp.take_along_axis(r, idx, axis=1))
        y = y * r_sel.reshape(B, C, 1)
        b_off = (jnp.arange(B) * S).reshape(B, 1)
        flat_idx = (idx + b_off).reshape(B * C)
        zero = (x * 0.0).reshape(B * S, D)
        upd = _scatter_add(zero, flat_idx, y.reshape(B * C, D), axis=0)
        return x + upd.reshape(B, S, D)

    x = A_x
    xn = _layernorm(x, axis=-1)
    return x + _A_ref(xn, A_wqkv, A_wo) + _B_ref(xn, B_w_r, B_w_gate, B_w_up, B_w_down)
```

```python
import functools
import jax
import jax.numpy as jnp
import numpy as np
from jax import lax
from jax.experimental import pallas as pl
from jax.experimental.pallas import tpu as pltpu

S, D, F, H, DH = 2048, 1024, 3584, 32, 32
f32, bf16, i32 = jnp.float32, jnp.bfloat16, jnp.int32

NN = (((1,), (0,)), ((), ()))
NT = (((1,), (1,)), ((), ()))
TN = (((0,), (0,)), ((), ()))


def mm(a, b, dims=NN):
    return lax.dot_general(a, b, dims, preferred_element_type=f32)


def rbf(v):
    u = pltpu.bitcast(v, jnp.uint32) if False else lax.bitcast_convert_type(v, jnp.uint32)
    u = (u + jnp.uint32(0x7FFF) + ((u >> 16) & jnp.uint32(1))) & jnp.uint32(0xFFFF0000)
    return lax.bitcast_convert_type(u, f32)


def phi(t):
    return jnp.where(t > 0, t + 1.0, jnp.exp(t)) + 1e-6


def make_kernel(cfg):
    NB = cfg.get("NB", 4)
    BS = S // NB
    LR = cfg.get("LR", 64)
    KN = cfg.get("KN", 512)
    GN = cfg.get("GN", 256)
    QT = cfg.get("QT", 512)
    OB = cfg.get("OB", 512)
    ON = cfg.get("ON", 512)

    def kernel(x_hbm, wqkv_hbm, wo_hbm, wr_hbm, wg_hbm, wu_hbm, wd_hbm, out_hbm,
               xbuf, xn_buf, pk_buf, oT_buf, wq_buf, wk_buf, wv_buf, wo_buf, wr_buf,
               wg_buf, wu_buf, wd_buf, wqT_buf, g_buf, m_buf, zb_buf, in_sems, out_sems):
        sem = iter(range(64))
        x_cp = [pltpu.make_async_copy(x_hbm.at[pl.ds(b * BS, BS), :], xbuf.at[pl.ds(b * BS, BS), :], in_sems.at[next(sem)])
                for b in range(NB)]
        wr_cp = pltpu.make_async_copy(wr_hbm, wr_buf, in_sems.at[next(sem)])
        wq_cp = pltpu.make_async_copy(wqkv_hbm.at[:, pl.ds(0, D)], wq_buf, in_sems.at[next(sem)])
        wk_cp = pltpu.make_async_copy(wqkv_hbm.at[:, pl.ds(D, D)], wk_buf, in_sems.at[next(sem)])
        wv_cp = pltpu.make_async_copy(wqkv_hbm.at[:, pl.ds(2 * D, D)], wv_buf, in_sems.at[next(sem)])
        wo_cp = pltpu.make_async_copy(wo_hbm, wo_buf, in_sems.at[next(sem)])
        wg_cp = pltpu.make_async_copy(wg_hbm, wg_buf, in_sems.at[next(sem)])
        wu_cp = pltpu.make_async_copy(wu_hbm, wu_buf, in_sems.at[next(sem)])
        wd_cp = pltpu.make_async_copy(wd_hbm, wd_buf, in_sems.at[next(sem)])
        x_cp[0].start(); wr_cp.start(); wk_cp.start()
        for b in range(1, NB):
            x_cp[b].start()
        wg_cp.start(); wu_cp.start(); wd_cp.start()
        wq_cp.start(); wv_cp.start(); wo_cp.start()

        wr_cp.wait()
        wr = wr_buf[...].astype(f32)
        eps = np.float32(jnp.bfloat16(1e-5)) if False else np.float32(np.float32(1e-5))
        best = None
        bidx = None
        zacc = None

        def ln_chunk(r0):
            nonlocal best, bidx
            x = xbuf[pl.ds(r0, LR), :].astype(f32)
            mean = jnp.sum(x, axis=1, keepdims=True) * (1.0 / D)
            d = x - mean
            var = jnp.sum(d * d, axis=1, keepdims=True) * (1.0 / D)
            t2 = rbf(rbf(var) + EPS_BF16)
            t3 = rbf(jnp.sqrt(t2))
            rinv = 1.0 / t3
            xn = d * rinv
            xn_buf[pl.ds(r0, LR), :] = xn.astype(bf16)
            r = rbf(jnp.sum(xn * wr, axis=1, keepdims=True))
            r = jnp.where(r == r, r, -jnp.inf)
            ridx = (lax.broadcasted_iota(i32, (LR, 1), 0) + r0).astype(f32)
            if best is None:
                best, bidx = r, ridx
            else:
                c = r > best
                best = jnp.where(c, r, best)
                bidx = jnp.where(c, ridx, bidx)

        for b in range(NB):
            x_cp[b].wait()
            for r0 in range(b * BS, (b + 1) * BS, LR):
                ln_chunk(r0)
            if b == 0:
                wk_cp.wait()
            xnb = xn_buf[pl.ds(b * BS, BS), :]
            for n0 in range(0, D, KN):
                pk = phi(mm(xnb, wk_buf[:, pl.ds(n0, KN)]))
                pk_buf[pl.ds(b * BS, BS), pl.ds(n0, KN)] = pk.astype(bf16)
                zp = jnp.sum(pk.reshape(BS // 8, 8, KN), axis=0)
                if b == 0:
                    zacc = zp if n0 == 0 else jnp.concatenate([zacc, zp], axis=1)
                else:
                    zacc = jnp.concatenate([zacc[:, :n0], zacc[:, n0:n0 + KN] + zp, zacc[:, n0 + KN:]], axis=1) if False else _addslab(zacc, zp, n0, KN)

        m = jnp.max(best)
        cand = jnp.where(best == m, bidx, np.float32(2 * S))
        idxf = jnp.min(cand)
        idx = jnp.clip(idxf.astype(i32), 0, S - 1)
        g0 = pl.multiple_of((idx // 16) * 16, 16)
        rows = xn_buf[pl.ds(g0, 16), :].astype(f32)
        sel = lax.broadcasted_iota(i32, (16, D), 0) == (idx - g0)
        xrow = jnp.sum(jnp.where(sel, rows, 0.0), axis=0, keepdims=True)
        x16 = jnp.broadcast_to(xrow, (16, D)).astype(bf16)
        rsel = rbf(jnp.sum(xrow * wr, axis=1, keepdims=True))
        gate = rbf(1.0 / (1.0 + jnp.exp(-rsel)))

        z = jnp.sum(zacc, axis=0, keepdims=True)
        zb_buf[...] = jnp.broadcast_to(z, (128, D)).T

        pk_all = pk_buf[...]
        for n0 in range(0, D, GN):
            g_buf[:, pl.ds(n0, GN)] = mm(pk_all, xn_buf[:, pl.ds(n0, GN)], TN).astype(bf16)

        wg_cp.wait(); wu_cp.wait()
        g = mm(x16, wg_buf[...])
        u = mm(x16, wu_buf[...])
        h = (g * (1.0 / (1.0 + jnp.exp(-g)))) * u
        wd_cp.wait()
        y = mm(h.astype(bf16), wd_buf[...])[0:1, :] * gate

        wv_cp.wait(); wo_cp.wait()
        rr = lax.broadcasted_iota(i32, (128, 128), 0) // DH
        cc = lax.broadcasted_iota(i32, (128, 128), 1) // DH
        bd = rr == cc
        for c in range(D // 128):
            kv = mm(g_buf[pl.ds(c * 128, 128), :], wv_buf[:, pl.ds(c * 128, 128)])
            kv = jnp.where(bd, kv, 0.0).astype(bf16)
            m_buf[pl.ds(c * 128, 128), :] = mm(kv, wo_buf[pl.ds(c * 128, 128), :]).astype(bf16)

        wq_cp.wait()
        wqT_buf[...] = wq_buf[...].T
        wqT = wqT_buf[...]
        zb = zb_buf[...]
        for t0 in range(0, S, QT):
            pq = phi(mm(wqT, xn_buf[pl.ds(t0, QT), :], NT))
            tz = jnp.concatenate([pq[:, j * 128:(j + 1) * 128] * zb for j in range(QT // 128)], axis=1)
            den = jnp.sum(tz.reshape(H, DH, QT), axis=1, keepdims=True) + 1e-6
            o = pq.reshape(H, DH, QT) * (1.0 / den)
            oT_buf[:, pl.ds(t0, QT)] = o.reshape(D, QT).astype(bf16)

        rows2 = jnp.where(sel, rows + rbf(y), rows)
        xn_buf[pl.ds(g0, 16), :] = rows2.astype(bf16)

        o_cp = []
        for bi, t0 in enumerate(range(0, S, OB)):
            ot = oT_buf[:, pl.ds(t0, OB)]
            for n0 in range(0, D, ON):
                acc = mm(ot, m_buf[:, pl.ds(n0, ON)], TN)
                res = xbuf[pl.ds(t0, OB), pl.ds(n0, ON)].astype(f32) + xn_buf[pl.ds(t0, OB), pl.ds(n0, ON)].astype(f32)
                xbuf[pl.ds(t0, OB), pl.ds(n0, ON)] = (acc + res).astype(bf16)
            cp = pltpu.make_async_copy(xbuf.at[pl.ds(t0, OB), :], out_hbm.at[pl.ds(t0, OB), :], out_sems.at[bi])
            cp.start()
            o_cp.append(cp)
        for cp in o_cp:
            cp.wait()

    return kernel, NB, S // OB


def _addslab(zacc, zp, n0, KN):
    parts = []
    if n0 > 0:
        parts.append(zacc[:, :n0])
    parts.append(zacc[:, n0:n0 + KN] + zp)
    if n0 + KN < zacc.shape[1]:
        parts.append(zacc[:, n0 + KN:])
    return jnp.concatenate(parts, axis=1) if len(parts) > 1 else parts[0]


EPS_BF16 = np.float32(1.0013580322265625e-05)


def build(cfg=None):
    cfg = cfg or {}
    kernel, nb, nob = make_kernel(cfg)
    anyspec = pl.BlockSpec(memory_space=pl.ANY)
    scratch = [
        pltpu.VMEM((S, D), bf16),
        pltpu.VMEM((S, D), bf16),
        pltpu.VMEM((S, D), bf16),
        pltpu.VMEM((D, S), bf16),
        pltpu.VMEM((D, D), bf16),
        pltpu.VMEM((D, D), bf16),
        pltpu.VMEM((D, D), bf16),
        pltpu.VMEM((D, D), bf16),
        pltpu.VMEM((1, D), bf16),
        pltpu.VMEM((D, F), bf16),
        pltpu.VMEM((D, F), bf16),
        pltpu.VMEM((F, D), bf16),
        pltpu.VMEM((D, D), bf16),
        pltpu.VMEM((D, D), bf16),
        pltpu.VMEM((D, D), bf16),
        pltpu.VMEM((D, 128), f32),
        pltpu.SemaphoreType.DMA((nb + 8,)),
        pltpu.SemaphoreType.DMA((nob,)),
    ]
    call = pl.pallas_call(
        kernel,
        out_shape=jax.ShapeDtypeStruct((S, D), bf16),
        in_specs=[anyspec] * 7,
        out_specs=anyspec,
        scratch_shapes=scratch,
        compiler_params=pltpu.CompilerParams(vmem_limit_bytes=cfg.get("VMEM", 110) * 2**20),
    )

    def fn(A_x, A_wqkv, A_wo, B_x, B_w_r, B_w_gate, B_w_up, B_w_down):
        out = call(A_x.reshape(S, D), A_wqkv, A_wo, B_w_r.reshape(1, D), B_w_gate, B_w_up, B_w_down)
        return out.reshape(1, S, D)

    return fn


_CFG = {}


@jax.jit
def pallas_parallel_sum__linear_attn_block__moe_arch_mod__prompt_kernel(
    A_x: jax.Array,
    A_wqkv: jax.Array,
    A_wo: jax.Array,
    B_x: jax.Array,
    B_w_r: jax.Array,
    B_w_gate: jax.Array,
    B_w_up: jax.Array,
    B_w_down: jax.Array,
):
    return build(_CFG)(A_x, A_wqkv, A_wo, B_x, B_w_r, B_w_gate, B_w_up, B_w_down)
```

```python
import contextlib
import jax
import jax.numpy as jnp
import numpy as np
from jax import lax
from jax.experimental import pallas as pl
from jax.experimental.pallas import tpu as pltpu

S, D, F, H, DH = 2048, 1024, 3584, 32, 32
f32, bf16, i32, u32 = jnp.float32, jnp.bfloat16, jnp.int32, jnp.uint32

NN = (((1,), (0,)), ((), ()))
NT = (((1,), (1,)), ((), ()))
EPS_BF16 = np.float32(1.0013580322265625e-05)


def mm(a, b, dims=NN):
    return lax.dot_general(a, b, dims, preferred_element_type=f32)


def rbf(v):
    return v.astype(bf16).astype(f32)


def phi(t):
    return jnp.where(t > 0, t + 1.0, jnp.exp(t)) + 1e-6


def bits(v):
    return pltpu.bitcast(v, u32)


def orall(vs):
    f = vs[0]
    for o in vs[1:]:
        f = f | o
    return f


def scope(cfg, name):
    return jax.named_scope(name) if cfg.get("SCOPES") else contextlib.nullcontext()


class Stream:
    def __init__(self, enable=True):
        self.Z = None
        self.i = 0
        self.res = {}
        self.pend = {}
        self.enable = enable
        self.bar = 0

    def tie(self, target, src_bits):
        tb = pltpu.bitcast(target, u32)
        return pltpu.bitcast(tb | (src_bits & self.Z), target.dtype)

    def dot(self, lhs, rhs, dims=NN, nk=4):
        fl = self.pend.pop(self.i, None)
        if fl and self.enable and self.Z is not None:
            f = orall(fl)
            K = lhs.shape[1]
            nk = min(nk, K // 128)
            parts = [self.tie(lhs[0:16, j * 128:(j + 1) * 128], f) for j in range(nk)]
            if nk * 128 < K:
                parts.append(lhs[0:16, nk * 128:])
            top = jnp.concatenate(parts, axis=1) if len(parts) > 1 else parts[0]
            lhs = jnp.concatenate([top, lhs[16:]], axis=0)
        p = mm(lhs, rhs, dims)
        m = p.shape[0]
        self.res[self.i] = p[m - 8:m, 0:128]
        self.i += 1
        return p

    def barrier(self):
        self.res = {}
        self.bar = self.i
        for k in [k for k in self.pend if k <= self.i]:
            pass

    def side(self, task, rel=1, dl=2):
        di = self.i - 1
        relbits = None
        if rel is not None and self.enable and self.Z is not None:
            relv = self.res.get(di - rel)
            if relv is not None:
                relbits = bits(relv)
        f = task(relbits)
        if f is not None and dl is not None:
            self.pend.setdefault(di + dl, []).append(f)

    def gate(self, v, relbits):
        if relbits is None:
            return v
        if v.shape == (8, 128):
            return self.tie(v, relbits)
        top = self.tie(v[0:8, 0:128], relbits)
        row = top if v.shape[1] == 128 else jnp.concatenate([top, v[0:8, 128:]], axis=1)
        return row if v.shape[0] == 8 else jnp.concatenate([row, v[8:]], axis=0)


def spread(ntasks, first, last):
    n = last - first
    out, done = {}, 0
    for s in range(n):
        upto = ntasks * (s + 1) // n
        out[first + s] = upto - done
        done = upto
    return out


def tile_bits_bf16(v):
    a, b = v.shape[0] // 128, v.shape[1] // 128
    return orall([bits(v[i * 128 + 112:(i + 1) * 128, j * 128:(j + 1) * 128]) for i in range(a) for j in range(b)])


def tile_bits_f32(v):
    a, b = v.shape[0] // 128, v.shape[1] // 128
    return orall([bits(v[i * 128 + 120:(i + 1) * 128, j * 128:(j + 1) * 128]) for i in range(a) for j in range(b)])


def make_kernel(cfg):
    LR = cfg.get("LR", 16)
    KM, KN = cfg.get("KM", 256), cfg.get("KN", 256)
    GK = cfg.get("GK", 512)
    GN = cfg.get("GN", 128)
    QT = cfg.get("QT", 128)
    ON = cfg.get("ON", 128)
    MOE = cfg.get("MOE", "vpu")
    MCOL, MROWS = cfg.get("MCOL", 7), cfg.get("MROWS", 256)
    DCOL, DROWS = cfg.get("DCOL", 8), cfg.get("DROWS", 256)
    G1 = cfg.get("G1", 11)
    Q1 = cfg.get("Q1", 3)
    REL, DL = cfg.get("REL", 1), cfg.get("DL", 2)
    NK = cfg.get("NK", 4)
    RR = cfg.get("RR", 64)
    NOUT = D // ON
    XP = cfg.get("XP", [256, 256, 256, 512, 768])

    def kernel(x_hbm, wqkv_hbm, wo_hbm, wr_hbm, wg_hbm, wu_hbm, wd_hbm, out_hbm,
               xbuf, xn_buf, pkT_buf, o_buf, wq_buf, wk_buf, wv_buf, wo_buf, wr_buf,
               wg_buf, wu_buf, wd_buf, wqT_buf, g_buf, m_buf, zb_buf, xb_buf, hb_buf, z2_buf, in_sems, out_sems):
        sem = iter(range(64))

        def cp(src, dst):
            return pltpu.make_async_copy(src, dst, in_sems.at[next(sem)])

        xs = [0]
        for n in XP:
            xs.append(xs[-1] + n)
        assert xs[-1] == S
        names = {"x%d" % i: cp(x_hbm.at[pl.ds(xs[i], XP[i]), :], xbuf.at[pl.ds(xs[i], XP[i]), :]) for i in range(len(XP))}
        names["z"] = cp(x_hbm.at[pl.ds(0, 16), pl.ds(0, 128)], z2_buf)
        names["wr"] = cp(wr_hbm, wr_buf)
        for j in range(4):
            names["q%d" % j] = cp(wqkv_hbm.at[:, pl.ds(D + j * 256, 256)], wk_buf.at[:, pl.ds(j * 256, 256)])
        names["wq"] = cp(wqkv_hbm.at[:, pl.ds(0, D)], wq_buf)
        names["wv"] = cp(wqkv_hbm.at[:, pl.ds(2 * D, D)], wv_buf)
        names["wo"] = cp(wo_hbm, wo_buf)
        names["wg"] = cp(wg_hbm, wg_buf)
        names["wu"] = cp(wu_hbm, wu_buf)
        names["wd"] = cp(wd_hbm, wd_buf)
        order = cfg.get("ORDER", "x0 x1 z q0 q1 x2 q2 q3 x3 wr x4 wq wg wu wv wo wd").split()
        assert sorted(order) == sorted(names)
        for nm in order:
            names[nm].start()

        st = Stream(cfg.get("TIE", True))

        def wait(lst):
            for nm in lst.split():
                with scope(cfg, "w_" + nm):
                    names[nm].wait()
            st.barrier()

        def ln_task(r0):
            def task(relbits):
                x = st.gate(xbuf[pl.ds(r0, LR), :].astype(f32), relbits)
                mean = jnp.sum(x, axis=1, keepdims=True) * (1.0 / D)
                d = x - mean
                var = jnp.sum(d * d, axis=1, keepdims=True) * (1.0 / D)
                t3 = rbf(jnp.sqrt(rbf(rbf(var) + EPS_BF16)))
                xn = d * (1.0 / t3)
                xn_buf[pl.ds(r0, LR), :] = xn.astype(bf16)
                return orall([bits(xn[g * 8:(g + 1) * 8, D - 128:D]) for g in range(LR // 8)])
            return task

        def ln_rows(a, b):
            for r0 in range(a, b, LR):
                ln_task(r0)(None)

        zacc = {}
        with scope(cfg, "stA"):
            nrb, ncb = S // KM, D // KN
            U = cfg.get("UNITS")
            if U is None:
                U = [(0, 0), (1, 0), (0, 1), (1, 1), (0, 2), (1, 2), (2, 0), (2, 1), (2, 2), (0, 3), (1, 3), (2, 3)]
                U += [(rb, cb) for rb in range(3, nrb) for cb in range(ncb)]
            assert sorted(U) == sorted((rb, cb) for rb in range(nrb) for cb in range(ncb))
            WA = cfg.get("WA", {0: "q0", 2: "q1", 4: "q2 x2", 9: "q3 x3", 16: "x4 wr wq"})
            first_use = {}
            for ui, (rb, cb) in enumerate(U):
                first_use.setdefault(rb, ui)
            wait("x0"); ln_rows(0, 256)
            wait("x1 z"); ln_rows(256, 512)
            st.Z = bits(z2_buf[...]) ^ bits(xbuf[0:16, 0:128])

            def avail(row):
                pc = max(i for i in range(len(XP)) if xs[i] <= row)
                if pc < 2:
                    return 0
                for ui in sorted(WA):
                    if ("x%d" % pc) in WA[ui].split():
                        return ui
                raise ValueError

            slots = {}
            for rb in range(512 // KM, nrb):
                tl = [ln_task(r) for r in range(rb * KM, (rb + 1) * KM, LR)]
                u_need = first_use[rb]
                u_first = max(avail(rb * KM), u_need - cfg.get("LNSPAN", 4))
                assert u_first < u_need, (rb, u_first, u_need)
                cnt = spread(len(tl), u_first, u_need)
                ti = 0
                for j in range(u_first, u_need):
                    for _ in range(cnt[j]):
                        slots.setdefault(j, []).append((tl[ti], u_need)); ti += 1

            def k_epilogue(rb, cb, p):
                def task(relbits):
                    pk = phi(p)
                    zp = jnp.sum(pk.reshape(KM // 8, 8, KN), axis=0)
                    zacc[cb] = zp if cb not in zacc else zacc[cb] + zp
                    pt = pk.astype(bf16).T
                    pkT_buf[pl.ds(cb * KN, KN), pl.ds(rb * KM, KM)] = pt
                    return tile_bits_bf16(pt)
                return task

            deferred = None
            for ui, (rb, cb) in enumerate(U):
                if ui in WA:
                    wait(WA[ui])
                p = st.dot(xn_buf[pl.ds(rb * KM, KM), :], wk_buf[:, pl.ds(cb * KN, KN)], nk=NK)
                if deferred is not None:
                    st.side(deferred, rel=None, dl=1); deferred = None
                nxtw = min([w for w in WA if w > ui] + [10 ** 9])
                ep = k_epilogue(rb, cb, p)
                if ui + 1 == nxtw and cfg.get("DEFER", True):
                    deferred = ep
                else:
                    st.side(ep, rel=None, dl=DL if ui + DL <= nxtw else (1 if ui + 1 < nxtw else None))
                for (t, u_need) in slots.get(ui, []):
                    dl = min(DL, u_need - ui, nxtw - ui)
                    if ui + dl >= nxtw:
                        dl = None if dl == nxtw - ui and ui + 1 >= nxtw else dl
                    st.side(t, rel=REL, dl=dl if (dl is None or ui + dl < nxtw or dl == nxtw - ui) else None)
            assert deferred is None

        rstate = {}

        def router_task(r0):
            def task(relbits):
                if "wr" not in rstate:
                    w8 = wr_buf[...].astype(f32)
                    rstate["wr"] = jnp.concatenate([w8[j:j + 1, :] for j in range(8)], axis=1)
                    rstate["best"] = jnp.full((RR, 1), -jnp.inf, f32)
                    rstate["bidx"] = jnp.zeros((RR, 1), f32)
                    rstate["iota"] = lax.broadcasted_iota(i32, (RR, 1), 0).astype(f32)
                xn = st.gate(xn_buf[pl.ds(r0, RR), :].astype(f32), relbits)
                pr = xn * rstate["wr"]
                sp = pr[:, 0:128]
                for j in range(1, D // 128):
                    sp = sp + pr[:, j * 128:(j + 1) * 128]
                r = rbf(jnp.sum(sp, axis=1, keepdims=True))
                c = r > rstate["best"]
                rstate["best"] = jnp.where(c, r, rstate["best"])
                rstate["bidx"] = jnp.where(c, rstate["iota"] + np.float32(r0), rstate["bidx"])
                return orall([bits(sp[g * 8:(g + 1) * 8]) for g in range(RR // 8)])
            return task

        sel = {}

        def router_final(relbits):
            best, bidx = rstate["best"], rstate["bidx"]
            m = jnp.max(best)
            cand = jnp.where(best == m, bidx, np.float32(2 * S))
            idx = jnp.clip(jnp.min(cand).astype(i32), 0, S - 1)
            g0 = pl.multiple_of((idx // 16) * 16, 16)
            rows = xn_buf[pl.ds(g0, 16), :].astype(f32)
            msk = lax.broadcasted_iota(i32, (16, D), 0) == (idx - g0)
            xrow = jnp.sum(jnp.where(msk, rows, 0.0), axis=0, keepdims=True)
            rsel = rbf(jnp.sum(xrow * rstate["wr"], axis=1, keepdims=True))
            sel.update(idx=idx, g0=g0, rows=rows, msk=msk, xrow=xrow, gate=rbf(1.0 / (1.0 + jnp.exp(-rsel))))
            if MOE == "vpu":
                xb = jnp.broadcast_to(xrow, (128, D)).T
                xb_buf[...] = xb
                return tile_bits_f32(xb)
            return None

        def zb_task(relbits):
            z = jnp.concatenate([jnp.sum(zacc[cb], axis=0, keepdims=True) for cb in range(D // KN)], axis=1)
            z = st.gate(jnp.broadcast_to(z, (8, D)), relbits)
            zb = jnp.broadcast_to(z[0:1], (128, D)).T
            zb_buf[...] = zb
            return tile_bits_f32(zb)

        def wqT_task(j):
            def task(relbits):
                w = wq_buf[:, pl.ds(j * 128, 128)]
                if relbits is not None:
                    w = jnp.concatenate([st.tie(w[0:16], relbits), w[16:]], axis=0)
                wt = w.T
                wqT_buf[pl.ds(j * 128, 128), :] = wt
                return tile_bits_bf16(wt)
            return task

        moe = {}

        def mv_tasks(w_ref, b_ref, K, ncolt, key, ncol, rows):
            ts = []
            for c0 in range(0, ncolt, ncol):
                state = {}
                for k0 in range(0, K, rows):
                    def task(relbits, c0=c0, k0=k0, state=state):
                        acc = state.get("acc")
                        for k in range(k0, k0 + rows, 16):
                            w = w_ref[k:k + 16, c0 * 128:(c0 + ncol) * 128].astype(f32)
                            xb = b_ref[k:k + 16, :]
                            if k == k0:
                                xb = st.gate(xb, relbits)
                            p = jnp.concatenate([w[:, j * 128:(j + 1) * 128] * xb for j in range(ncol)], axis=1)
                            p = p[0:8] + p[8:16]
                            acc = p if acc is None else acc + p
                        state["acc"] = acc
                        if k0 + rows == K:
                            moe[(key, c0)] = jnp.sum(acc, axis=0, keepdims=True)
                        return orall([bits(acc[:, j * 128:(j + 1) * 128]) for j in range(ncol)])
                    ts.append(task)
            return ts

        def hb_task(c0):
            def task(relbits):
                g = st.gate(jnp.broadcast_to(moe[("g", c0)], (8, MCOL * 128)), relbits)[0:1]
                u = moe[("u", c0)]
                g = rbf(g)
                h = rbf(rbf(g * (1.0 / (1.0 + jnp.exp(-g)))) * rbf(u))
                hb = jnp.broadcast_to(h, (128, MCOL * 128)).T
                hb_buf[pl.ds(c0 * 128, MCOL * 128), :] = hb
                return tile_bits_f32(hb)
            return task

        with scope(cfg, "stG"):
            nsub = (D // GN) * (S // GK)
            pre = [router_task(r) for r in range(0, S, RR)] + [router_final, zb_task] + [wqT_task(j) for j in range(D // 128)]
            post = []
            if MOE == "vpu":
                post = mv_tasks(wg_buf, xb_buf, D, F // 128, "g", MCOL, MROWS) + mv_tasks(wu_buf, xb_buf, D, F // 128, "u", MCOL, MROWS)
            c_pre = spread(len(pre), 0, G1 - 1)
            c_post = spread(len(post), G1, nsub - cfg.get("GEND", 1))
            pi = qi = di = 0
            for n in range(D // GN):
                acc = None
                for kc in range(S // GK):
                    if di == G1:
                        wait(cfg.get("WG1", "wg wu"))
                    p = st.dot(pkT_buf[:, pl.ds(kc * GK, GK)], xn_buf[pl.ds(kc * GK, GK), pl.ds(n * GN, GN)], nk=NK)
                    acc = p if acc is None else acc + p
                    if kc == S // GK - 1:
                        g_buf[:, pl.ds(n * GN, GN)] = acc.astype(bf16)
                    for _ in range(c_pre.get(di, 0)):
                        st.side(pre[pi], rel=REL, dl=min(DL, G1 - 1 - di)); pi += 1
                    for _ in range(c_post.get(di, 0)):
                        st.side(post[qi], rel=REL, dl=DL if di + DL <= nsub else 1); qi += 1
                    di += 1
            assert pi == len(pre) and qi == len(post)

        with scope(cfg, "stQ"):
            td = mv_tasks(wd_buf, hb_buf, F, D // 128, "d", DCOL, DROWS) if MOE == "vpu" else []
            rr = lax.broadcasted_iota(i32, (128, 128), 0) // DH
            cc = lax.broadcasted_iota(i32, (128, 128), 1) // DH
            bd = rr == cc

            def chain_task(c):
                def task(relbits):
                    kv = mm(g_buf[pl.ds(c * 128, 128), :], wv_buf[:, pl.ds(c * 128, 128)])
                    kv = jnp.where(bd, kv, 0.0).astype(bf16)
                    m_buf[pl.ds(c * 128, 128), :] = mm(kv, wo_buf[pl.ds(c * 128, 128), :]).astype(bf16)
                    return None
                return task

            def q_epilogue(t0, q):
                def task(relbits):
                    pq = phi(q)
                    zb = zb_buf[...]
                    tz = jnp.concatenate([pq[:, j * 128:(j + 1) * 128] * zb for j in range(QT // 128)], axis=1) if QT > 128 else pq * zb
                    den = jnp.sum(tz.reshape(H, DH, QT), axis=1, keepdims=True) + 1e-6
                    o = (pq.reshape(H, DH, QT) * (1.0 / den)).reshape(D, QT)
                    ot = o.astype(bf16).T
                    o_buf[pl.ds(t0, QT), :] = ot
                    return tile_bits_bf16(ot)
                return task

            nq = S // QT
            hbt = [hb_task(c0) for c0 in range(0, F // 128, MCOL)] if MOE == "vpu" else []
            c_hb = spread(len(hbt), 0, max(1, Q1 - 1))
            chain = [chain_task(c) for c in range(D // 128)]
            c_chain = spread(len(chain), Q1, min(nq, Q1 + cfg.get("CHN", 8)))
            c_down = spread(len(td), Q1, nq - cfg.get("DEND", 1))
            ci = dni = hi = 0
            deferred = None
            for qd in range(nq):
                t0 = qd * QT
                if qd == Q1:
                    wait("wv wo wd")
                    if MOE != "vpu":
                        x16 = jnp.broadcast_to(sel["xrow"], (16, D)).astype(bf16)
                        g = rbf(mm(x16, wg_buf[...]))
                        u = rbf(mm(x16, wu_buf[...]))
                        h = rbf(g * (1.0 / (1.0 + jnp.exp(-g)))) * u
                        ymx = mm(h.astype(bf16), wd_buf[...])[0:1, :]
                q = st.dot(wqT_buf[...], xn_buf[pl.ds(t0, QT), :], NT, nk=NK)
                if deferred is not None:
                    st.side(deferred, rel=None, dl=1); deferred = None
                ep = q_epilogue(t0, q)
                if qd + 1 == Q1 and cfg.get("DEFER", True):
                    deferred = ep
                else:
                    st.side(ep, rel=None, dl=cfg.get("QEDL", DL) if (qd + DL < nq and not (qd < Q1 <= qd + DL)) else (1 if (qd + 1 < nq and qd + 1 != Q1) else None))
                for _ in range(c_hb.get(qd, 0)):
                    st.side(hbt[hi], rel=REL, dl=min(DL, Q1 - qd) if Q1 - qd >= 2 else None); hi += 1
                for _ in range(c_chain.get(qd, 0)):
                    st.side(chain[ci], rel=None, dl=None); ci += 1
                for _ in range(c_down.get(qd, 0)):
                    st.side(td[dni], rel=REL, dl=DL if qd + DL < nq else (1 if qd + 1 < nq else None)); dni += 1
            assert ci == len(chain) and dni == len(td) and hi == len(hbt) and deferred is None
            if MOE == "vpu":
                y = jnp.concatenate([moe[("d", c0)] for c0 in range(0, D // 128, DCOL)], axis=1)
            else:
                y = ymx
            y = rbf(rbf(y) * sel["gate"])
            rows2 = jnp.where(sel["msk"], sel["rows"] + y, sel["rows"])
            xn_buf[pl.ds(sel["g0"], 16), :] = rows2.astype(bf16)

        with scope(cfg, "stD"):
            o_cp = []
            for n in range(NOUT):
                n0 = n * ON
                acc = st.dot(o_buf[...], m_buf[:, pl.ds(n0, ON)], nk=NK)
                res = xbuf[:, pl.ds(n0, ON)].astype(f32) + xn_buf[:, pl.ds(n0, ON)].astype(f32)
                xbuf[:, pl.ds(n0, ON)] = (acc + res).astype(bf16)
                c = pltpu.make_async_copy(xbuf.at[:, pl.ds(n0, ON)], out_hbm.at[:, pl.ds(n0, ON)], out_sems.at[n])
                c.start()
                o_cp.append(c)
            for c in o_cp:
                c.wait()

    return kernel, len(XP) + 12, NOUT


def build(cfg=None):
    cfg = cfg or {}
    kernel, nin, nout = make_kernel(cfg)
    anyspec = pl.BlockSpec(memory_space=pl.ANY)
    scratch = [
        pltpu.VMEM((S, D), bf16),
        pltpu.VMEM((S, D), bf16),
        pltpu.VMEM((D, S), bf16),
        pltpu.VMEM((S, D), bf16),
        pltpu.VMEM((D, D), bf16),
        pltpu.VMEM((D, D), bf16),
        pltpu.VMEM((D, D), bf16),
        pltpu.VMEM((D, D), bf16),
        pltpu.VMEM((8, 128), bf16),
        pltpu.VMEM((D, F), bf16),
        pltpu.VMEM((D, F), bf16),
        pltpu.VMEM((F, D), bf16),
        pltpu.VMEM((D, D), bf16),
        pltpu.VMEM((D, D), bf16),
        pltpu.VMEM((D, D), bf16),
        pltpu.VMEM((D, 128), f32),
        pltpu.VMEM((D, 128), f32),
        pltpu.VMEM((F, 128), f32),
        pltpu.VMEM((16, 128), bf16),
        pltpu.SemaphoreType.DMA((nin,)),
        pltpu.SemaphoreType.DMA((nout,)),
    ]
    call = pl.pallas_call(
        kernel,
        out_shape=jax.ShapeDtypeStruct((S, D), bf16),
        in_specs=[anyspec] * 7,
        out_specs=anyspec,
        scratch_shapes=scratch,
        compiler_params=pltpu.CompilerParams(vmem_limit_bytes=cfg.get("VMEM", 110) * 2**20),
        interpret=cfg.get("INTERPRET", False),
    )

    def fn(A_x, A_wqkv, A_wo, B_x, B_w_r, B_w_gate, B_w_up, B_w_down):
        out = call(A_x.reshape(S, D), A_wqkv, A_wo, B_w_r.reshape(8, 128), B_w_gate, B_w_up, B_w_down)
        return out.reshape(1, S, D)

    return fn


_CFG = {}


@jax.jit
def pallas_parallel_sum__linear_attn_block__moe_arch_mod__prompt_kernel(
    A_x: jax.Array,
    A_wqkv: jax.Array,
    A_wo: jax.Array,
    B_x: jax.Array,
    B_w_r: jax.Array,
    B_w_gate: jax.Array,
    B_w_up: jax.Array,
    B_w_down: jax.Array,
):
    return build(_CFG)(A_x, A_wqkv, A_wo, B_x, B_w_r, B_w_gate, B_w_up, B_w_down)
```

```python
import contextlib
import jax
import jax.numpy as jnp
import numpy as np
from jax import lax
from jax.experimental import pallas as pl
from jax.experimental.pallas import tpu as pltpu

S, D, F, H, DH = 2048, 1024, 3584, 32, 32
f32, bf16, i32, u32 = jnp.float32, jnp.bfloat16, jnp.int32, jnp.uint32

NN = (((1,), (0,)), ((), ()))
NT = (((1,), (1,)), ((), ()))
EPS_BF16 = np.float32(1.0013580322265625e-05)


def mm(a, b, dims=NN):
    return lax.dot_general(a, b, dims, preferred_element_type=f32)


def rbf(v):
    return v.astype(bf16).astype(f32)


def phi(t):
    return jnp.where(t > 0, t + 1.0, jnp.exp(t)) + 1e-6


def bits(v):
    return pltpu.bitcast(v, u32)


def orall(vs):
    f = vs[0]
    for o in vs[1:]:
        f = f | o
    return f


def scope(cfg, name):
    return jax.named_scope(name) if cfg.get("SCOPES") else contextlib.nullcontext()


class Stream:
    def __init__(self, enable=True):
        self.Z = None
        self.i = 0
        self.res = {}
        self.pend = {}
        self.enable = enable
        self.bar = 0

    def tie(self, target, src_bits):
        tb = pltpu.bitcast(target, u32)
        return pltpu.bitcast(tb | (src_bits & self.Z), target.dtype)

    def dot(self, lhs, rhs, dims=NN, nk=4, tie_row=0):
        fl = self.pend.pop(self.i, None)
        if fl and self.enable and self.Z is not None:
            f = orall(fl)
            K = lhs.shape[1]
            nk = min(nk, K // 128)
            r = tie_row
            parts = [self.tie(lhs[r:r + 16, j * 128:(j + 1) * 128], f) for j in range(nk)]
            if nk * 128 < K:
                parts.append(lhs[r:r + 16, nk * 128:])
            top = jnp.concatenate(parts, axis=1) if len(parts) > 1 else parts[0]
            lhs = jnp.concatenate(([lhs[:r]] if r else []) + [top, lhs[r + 16:]], axis=0)
        p = mm(lhs, rhs, dims)
        m = p.shape[0]
        self.res[self.i] = p[m - 8:m, 0:128]
        self.i += 1
        return p

    def barrier(self):
        self.res = {}
        self.bar = self.i
        for k in [k for k in self.pend if k <= self.i]:
            pass

    def side(self, task, rel=1, dl=2):
        di = self.i - 1
        relbits = None
        if rel is not None and self.enable and self.Z is not None:
            relv = self.res.get(di - rel)
            if relv is not None:
                relbits = bits(relv)
        f = task(relbits)
        if f is not None and dl is not None:
            self.pend.setdefault(di + dl, []).append(f)

    def gate(self, v, relbits):
        if relbits is None:
            return v
        if v.shape == (8, 128):
            return self.tie(v, relbits)
        top = self.tie(v[0:8, 0:128], relbits)
        row = top if v.shape[1] == 128 else jnp.concatenate([top, v[0:8, 128:]], axis=1)
        return row if v.shape[0] == 8 else jnp.concatenate([row, v[8:]], axis=0)


def gate_all(st, v, relbits):
    if relbits is None:
        return v
    rows = []
    for i in range(v.shape[0] // 8):
        cols = [st.tie(v[i * 8:(i + 1) * 8, j * 128:(j + 1) * 128], relbits) for j in range(v.shape[1] // 128)]
        rows.append(jnp.concatenate(cols, axis=1) if len(cols) > 1 else cols[0])
    return jnp.concatenate(rows, axis=0) if len(rows) > 1 else rows[0]


def spread(ntasks, first, last):
    n = last - first
    out, done = {}, 0
    for s in range(n):
        upto = ntasks * (s + 1) // n
        out[first + s] = upto - done
        done = upto
    return out


def tile_bits_bf16(v):
    a, b = v.shape[0] // 128, v.shape[1] // 128
    return orall([bits(v[i * 128 + 112:(i + 1) * 128, j * 128:(j + 1) * 128]) for i in range(a) for j in range(b)])


def tile_bits_f32(v):
    a, b = v.shape[0] // 128, v.shape[1] // 128
    return orall([bits(v[i * 128 + 120:(i + 1) * 128, j * 128:(j + 1) * 128]) for i in range(a) for j in range(b)])


def make_kernel(cfg):
    LR = cfg.get("LR", 16)
    KM, KN = cfg.get("KM", 256), cfg.get("KN", 256)
    GK = cfg.get("GK", 512)
    GN = cfg.get("GN", 128)
    QT = cfg.get("QT", 128)
    ON = cfg.get("ON", 128)
    MOE = cfg.get("MOE", "vpu")
    MCOL, MROWS = cfg.get("MCOL", 7), cfg.get("MROWS", 256)
    DCOL, DROWS = cfg.get("DCOL", 8), cfg.get("DROWS", 256)
    G1 = cfg.get("G1", 11)
    Q1 = cfg.get("Q1", 3)
    REL, DL = cfg.get("REL", 1), cfg.get("DL", 2)
    NK = cfg.get("NK", 4)
    RR = cfg.get("RR", 64)
    NOUT = D // ON
    DTAIL = cfg.get("DTAIL", 4)
    XP = cfg.get("XP", [256, 256, 256, 512, 768])

    def kernel(x_hbm, wqkv_hbm, wo_hbm, wr_hbm, wg_hbm, wu_hbm, wd_hbm, out_hbm,
               xbuf, xn_buf, pkT_buf, o_buf, wq_buf, wk_buf, wv_buf, wo_buf, wr_buf,
               wg_buf, wu_buf, wd_buf, wqT_buf, g_buf, m_buf, zb_buf, xb_buf, hb_buf, z2_buf, in_sems, out_sems):
        sem = iter(range(64))

        def cp(src, dst):
            return pltpu.make_async_copy(src, dst, in_sems.at[next(sem)])

        xs = [0]
        for n in XP:
            xs.append(xs[-1] + n)
        assert xs[-1] == S
        names = {"x%d" % i: cp(x_hbm.at[pl.ds(xs[i], XP[i]), :], xbuf.at[pl.ds(xs[i], XP[i]), :]) for i in range(len(XP))}
        names["z"] = cp(x_hbm.at[pl.ds(0, 16), pl.ds(0, 128)], z2_buf)
        names["wr"] = cp(wr_hbm, wr_buf)
        for j in range(4):
            names["q%d" % j] = cp(wqkv_hbm.at[:, pl.ds(D + j * 256, 256)], wk_buf.at[:, pl.ds(j * 256, 256)])
        names["wq"] = cp(wqkv_hbm.at[:, pl.ds(0, D)], wq_buf)
        names["wv"] = cp(wqkv_hbm.at[:, pl.ds(2 * D, D)], wv_buf)
        names["wo"] = cp(wo_hbm, wo_buf)
        names["wg"] = cp(wg_hbm, wg_buf)
        names["wu"] = cp(wu_hbm, wu_buf)
        names["wd"] = cp(wd_hbm, wd_buf)
        order = cfg.get("ORDER", "x0 x1 z q0 q1 x2 q2 q3 x3 wr x4 wq wg wu wv wo wd").split()
        assert sorted(order) == sorted(names)
        for nm in order:
            names[nm].start()

        st = Stream(cfg.get("TIE", True))

        def wait(lst):
            for nm in lst.split():
                with scope(cfg, "w_" + nm):
                    names[nm].wait()
            st.barrier()

        def ln_task(r0):
            def task(relbits):
                x = st.gate(xbuf[pl.ds(r0, LR), :].astype(f32), relbits)
                mean = jnp.sum(x, axis=1, keepdims=True) * (1.0 / D)
                d = x - mean
                var = jnp.sum(d * d, axis=1, keepdims=True) * (1.0 / D)
                t3 = rbf(jnp.sqrt(rbf(rbf(var) + EPS_BF16)))
                xn = d * (1.0 / t3)
                xn_buf[pl.ds(r0, LR), :] = xn.astype(bf16)
                return orall([bits(xn[g * 8:(g + 1) * 8, D - 128:D]) for g in range(LR // 8)])
            return task

        def ln_rows(a, b):
            for r0 in range(a, b, LR):
                ln_task(r0)(None)

        zacc = {}
        with scope(cfg, "stA"):
            nrb, ncb = S // KM, D // KN
            U = cfg.get("UNITS")
            if U is None:
                U = [(0, 0), (1, 0), (0, 1), (1, 1), (0, 2), (1, 2), (2, 0), (2, 1), (2, 2), (0, 3), (1, 3), (2, 3)]
                U += [(rb, cb) for rb in range(3, nrb) for cb in range(ncb)]
            assert sorted(U) == sorted((rb, cb) for rb in range(nrb) for cb in range(ncb))
            WA = cfg.get("WA", {0: "q0", 2: "q1", 4: "q2 x2", 9: "q3 x3", 16: "x4 wr wq"})
            first_use = {}
            for ui, (rb, cb) in enumerate(U):
                first_use.setdefault(rb, ui)
            wait("x0"); ln_rows(0, 256)
            wait("x1 z"); ln_rows(256, 512)
            st.Z = bits(z2_buf[...]) ^ bits(xbuf[0:16, 0:128])

            def avail(row):
                pc = max(i for i in range(len(XP)) if xs[i] <= row)
                if pc < 2:
                    return 0
                for ui in sorted(WA):
                    if ("x%d" % pc) in WA[ui].split():
                        return ui
                raise ValueError

            slots = {}
            for rb in range(512 // KM, nrb):
                tl = [ln_task(r) for r in range(rb * KM, (rb + 1) * KM, LR)]
                u_need = first_use[rb]
                u_first = max(avail(rb * KM), u_need - cfg.get("LNSPAN", 4))
                u_last = u_need
                if cfg.get("LNGAP", False) and u_need in WA and u_need - u_first >= 2:
                    u_last = u_need - 1
                if rb in cfg.get("LNS", {}):
                    u_first, u_last = cfg["LNS"][rb]
                assert u_first < u_last <= u_need and u_first >= avail(rb * KM), (rb, u_first, u_need)
                cnt = spread(len(tl), u_first, u_last)
                ti = 0
                for j in range(u_first, u_last):
                    for _ in range(cnt[j]):
                        slots.setdefault(j, []).append((tl[ti], u_need)); ti += 1

            def k_epilogue(rb, cb, p):
                def task(relbits):
                    pk = phi(p)
                    zp = jnp.sum(pk.reshape(KM // 8, 8, KN), axis=0)
                    zacc[cb] = zp if cb not in zacc else zacc[cb] + zp
                    pt = pk.astype(bf16).T
                    pkT_buf[pl.ds(cb * KN, KN), pl.ds(rb * KM, KM)] = pt
                    return tile_bits_bf16(pt)
                return task

            deferred = None
            for ui, (rb, cb) in enumerate(U):
                if ui in WA:
                    wait(WA[ui])
                p = st.dot(xn_buf[pl.ds(rb * KM, KM), :], wk_buf[:, pl.ds(cb * KN, KN)], nk=NK)
                nxtw = min([w for w in WA if w > ui] + [10 ** 9])
                if deferred is not None:
                    DD = cfg.get("DEFDL", 2)
                    st.side(deferred, rel=None, dl=DD if ui + DD < nxtw else None); deferred = None
                ep = k_epilogue(rb, cb, p)
                if ui + 1 == nxtw and cfg.get("DEFER", True):
                    deferred = ep
                else:
                    KE = cfg.get("KEDL", DL)
                    st.side(ep, rel=None, dl=KE if ui + KE < nxtw else None)
                for (t, u_need) in slots.get(ui, []):
                    dl = min(cfg.get("LNDL", DL), u_need - ui)
                    st.side(t, rel=cfg.get("LNREL", REL), dl=dl if ui + dl < nxtw else None)
            assert deferred is None

        rstate = {}

        def router_task(r0):
            def task(relbits):
                if "wr" not in rstate:
                    w8 = wr_buf[...].astype(f32)
                    rstate["wr"] = jnp.concatenate([w8[j:j + 1, :] for j in range(8)], axis=1)
                    rstate["best"] = jnp.full((RR, 1), -jnp.inf, f32)
                    rstate["bidx"] = jnp.zeros((RR, 1), f32)
                    rstate["iota"] = lax.broadcasted_iota(i32, (RR, 1), 0).astype(f32)
                xn = st.gate(xn_buf[pl.ds(r0, RR), :].astype(f32), relbits)
                pr = xn * rstate["wr"]
                sp = pr[:, 0:128]
                for j in range(1, D // 128):
                    sp = sp + pr[:, j * 128:(j + 1) * 128]
                r = rbf(jnp.sum(sp, axis=1, keepdims=True))
                c = r > rstate["best"]
                rstate["best"] = jnp.where(c, r, rstate["best"])
                rstate["bidx"] = jnp.where(c, rstate["iota"] + np.float32(r0), rstate["bidx"])
                return orall([bits(sp[g * 8:(g + 1) * 8]) for g in range(RR // 8)])
            return task

        sel = {}

        def router_final(relbits):
            best, bidx = rstate["best"], rstate["bidx"]
            m = jnp.max(best)
            cand = jnp.where(best == m, bidx, np.float32(2 * S))
            idx = jnp.clip(jnp.min(cand).astype(i32), 0, S - 1)
            g0 = pl.multiple_of((idx // 16) * 16, 16)
            rows = xn_buf[pl.ds(g0, 16), :].astype(f32)
            msk = lax.broadcasted_iota(i32, (16, D), 0) == (idx - g0)
            xrow = jnp.sum(jnp.where(msk, rows, 0.0), axis=0, keepdims=True)
            rsel = rbf(jnp.sum(xrow * rstate["wr"], axis=1, keepdims=True))
            sel.update(idx=idx, g0=g0, rows=rows, msk=msk, xrow=xrow, gate=rbf(1.0 / (1.0 + jnp.exp(-rsel))))
            if MOE == "vpu":
                xb = jnp.broadcast_to(xrow, (128, D)).T
                xb_buf[...] = xb
                return tile_bits_f32(xb)
            return None

        def zb_task(relbits):
            z = jnp.concatenate([jnp.sum(zacc[cb], axis=0, keepdims=True) for cb in range(D // KN)], axis=1)
            z = st.gate(jnp.broadcast_to(z, (8, D)), relbits)
            zb = jnp.broadcast_to(z[0:1], (128, D)).T
            zb_buf[...] = zb
            return tile_bits_f32(zb)

        def wqT_task(j):
            def task(relbits):
                w = wq_buf[:, pl.ds(j * 128, 128)]
                if relbits is not None:
                    w = jnp.concatenate([st.tie(w[0:16], relbits), w[16:]], axis=0)
                wt = w.T
                wqT_buf[pl.ds(j * 128, 128), :] = wt
                return tile_bits_bf16(wt)
            return task

        moe = {}

        def mv_tasks(w_ref, b_ref, K, ncolt, key, ncol, rows):
            ts = []
            for c0 in range(0, ncolt, ncol):
                state = {}
                for k0 in range(0, K, rows):
                    def task(relbits, c0=c0, k0=k0, state=state):
                        acc = state.get("acc")
                        for k in range(k0, k0 + rows, 16):
                            w = w_ref[k:k + 16, c0 * 128:(c0 + ncol) * 128].astype(f32)
                            xb = b_ref[k:k + 16, :]
                            if (k - k0) % cfg.get("MGATE", 10 ** 6) == 0:
                                xb = gate_all(st, xb, relbits) if cfg.get("MGATEALL", False) else st.gate(xb, relbits)
                            p = jnp.concatenate([w[:, j * 128:(j + 1) * 128] * xb for j in range(ncol)], axis=1)
                            p = p[0:8] + p[8:16]
                            acc = p if acc is None else acc + p
                        state["acc"] = acc
                        if k0 + rows == K:
                            moe[(key, c0)] = jnp.sum(acc, axis=0, keepdims=True)
                        return orall([bits(acc[:, j * 128:(j + 1) * 128]) for j in range(ncol)])
                    ts.append(task)
            return ts

        def hb_task(c0):
            def task(relbits):
                g = gate_all(st, jnp.broadcast_to(moe[("g", c0)], (8, MCOL * 128)), relbits)[0:1]
                u = moe[("u", c0)]
                g = rbf(g)
                h = rbf(rbf(g * (1.0 / (1.0 + jnp.exp(-g)))) * rbf(u))
                hb = jnp.broadcast_to(h, (128, MCOL * 128)).T
                hb_buf[pl.ds(c0 * 128, MCOL * 128), :] = hb
                return tile_bits_f32(hb)
            return task

        with scope(cfg, "stG"):
            nsub = (D // GN) * (S // GK)
            wqt = [wqT_task(j) for j in range(D // 128)]
            pre = [router_task(r) for r in range(0, S, RR)] + [router_final, zb_task] + (wqt if cfg.get("WQT_PRE", True) else [])
            post = []
            nhb_g = 0
            if MOE == "vpu":
                tg = mv_tasks(wg_buf, xb_buf, D, F // 128, "g", MCOL, MROWS)
                tu = mv_tasks(wu_buf, xb_buf, D, F // 128, "u", MCOL, MROWS)
                per = D // MROWS
                ngrp = len(tg) // per
                if cfg.get("POSTMIX", True):
                    HBLAG = cfg.get("HBLAG", 2)
                    hbq = []
                    for gi in range(ngrp):
                        for j, t in enumerate(tg[gi * per:(gi + 1) * per] + tu[gi * per:(gi + 1) * per]):
                            post.append(t)
                            if j == HBLAG - 1 and hbq:
                                post.append(hbq.pop(0)); nhb_g += 1
                        hbq.append(hb_task(gi * MCOL))
                else:
                    post = tg + tu
            if not cfg.get("WQT_PRE", True):
                post = wqt + post
            c_pre = spread(len(pre), 0, G1 - 1)
            c_post = spread(len(post), G1, nsub - cfg.get("GEND", 1))
            pi = qi = di = 0
            for n in range(D // GN):
                acc = None
                for kc in range(S // GK):
                    if di == G1:
                        wait(cfg.get("WG1", "wg wu"))
                    p = st.dot(pkT_buf[:, pl.ds(kc * GK, GK)], xn_buf[pl.ds(kc * GK, GK), pl.ds(n * GN, GN)], nk=NK)
                    acc = p if acc is None else acc + p
                    if kc == S // GK - 1:
                        g_buf[:, pl.ds(n * GN, GN)] = acc.astype(bf16)
                    for _ in range(c_pre.get(di, 0)):
                        PD = cfg.get("PREDL", DL)
                        st.side(pre[pi], rel=cfg.get("PREREL", REL), dl=PD if di + PD < G1 else None); pi += 1
                    for _ in range(c_post.get(di, 0)):
                        st.side(post[qi], rel=cfg.get("MREL", REL), dl=cfg.get("MDL", DL)); qi += 1
                    di += 1
            assert pi == len(pre) and qi == len(post)

        with scope(cfg, "stQ"):
            td = mv_tasks(wd_buf, hb_buf, F, D // 128, "d", DCOL, DROWS) if MOE == "vpu" else []
            rr = lax.broadcasted_iota(i32, (128, 128), 0) // DH
            cc = lax.broadcasted_iota(i32, (128, 128), 1) // DH
            bd = rr == cc

            def chain_task(c):
                def task(relbits):
                    kv = mm(g_buf[pl.ds(c * 128, 128), :], wv_buf[:, pl.ds(c * 128, 128)])
                    kv = jnp.where(bd, kv, 0.0).astype(bf16)
                    m_buf[pl.ds(c * 128, 128), :] = mm(kv, wo_buf[pl.ds(c * 128, 128), :]).astype(bf16)
                    return None
                return task

            kvs = {}

            def kv_task(c):
                def task(relbits):
                    kv = mm(g_buf[pl.ds(c * 128, 128), :], wv_buf[:, pl.ds(c * 128, 128)])
                    kvs[c] = jnp.where(bd, kv, 0.0).astype(bf16)
                    return None
                return task

            def m_task(c):
                def task(relbits):
                    m_buf[pl.ds(c * 128, 128), :] = mm(kvs[c], wo_buf[pl.ds(c * 128, 128), :]).astype(bf16)
                    return None
                return task

            def q_epilogue(t0, q):
                def task(relbits):
                    pq = phi(q)
                    zb = zb_buf[...]
                    tz = jnp.concatenate([pq[:, j * 128:(j + 1) * 128] * zb for j in range(QT // 128)], axis=1) if QT > 128 else pq * zb
                    den = jnp.sum(tz.reshape(H, DH, QT), axis=1, keepdims=True) + 1e-6
                    o = (pq.reshape(H, DH, QT) * (1.0 / den)).reshape(D, QT)
                    ot = o.astype(bf16).T
                    o_buf[pl.ds(t0, QT), :] = ot
                    return tile_bits_bf16(ot)
                return task

            nq = S // QT
            hbt = [hb_task(c0) for c0 in range(0, F // 128, MCOL)][nhb_g:] if MOE == "vpu" else []
            c_hb = spread(len(hbt), cfg.get("HB0", 0), max(cfg.get("HB0", 0) + 1, Q1 - 1))
            chain = [chain_task(c) for c in range(D // 128)]
            c_chain = spread(len(chain), Q1 + cfg.get("CH0", 0), min(nq, Q1 + cfg.get("CH0", 0) + cfg.get("CHN", 8)))
            CHS = cfg.get("CHSPLIT", 0)
            mq = {}
            c_down = spread(len(td), Q1, nq - cfg.get("DEND", 1))
            ci = dni = hi = 0
            deferred = None
            for qd in range(nq):
                t0 = qd * QT
                if qd == Q1:
                    wait("wv wo wd")
                    if MOE != "vpu":
                        x16 = jnp.broadcast_to(sel["xrow"], (16, D)).astype(bf16)
                        g = rbf(mm(x16, wg_buf[...]))
                        u = rbf(mm(x16, wu_buf[...]))
                        h = rbf(g * (1.0 / (1.0 + jnp.exp(-g)))) * u
                        ymx = mm(h.astype(bf16), wd_buf[...])[0:1, :]
                q = st.dot(wqT_buf[...], xn_buf[pl.ds(t0, QT), :], NT, nk=NK)
                if deferred is not None:
                    st.side(deferred, rel=None, dl=cfg.get("DEFDL", 2)); deferred = None
                ep = q_epilogue(t0, q)
                if qd + 1 == Q1 and cfg.get("DEFER", True):
                    deferred = ep
                else:
                    QE = cfg.get("QEDL", DL)
                    st.side(ep, rel=None, dl=QE if (not (qd < Q1 <= qd + QE) and qd + QE < nq + cfg.get("QTAIL", 2)) else None)
                for _ in range(c_hb.get(qd, 0)):
                    st.side(hbt[hi], rel=REL, dl=DL if qd + DL < Q1 else None); hi += 1
                for c in mq.pop(qd, []):
                    st.side(m_task(c), rel=None, dl=None)
                for _ in range(c_chain.get(qd, 0)):
                    if CHS:
                        st.side(kv_task(ci), rel=None, dl=None); mq.setdefault(min(qd + CHS, nq - 1), []).append(ci)
                    else:
                        st.side(chain[ci], rel=None, dl=None)
                    ci += 1
                for _ in range(c_down.get(qd, 0)):
                    st.side(td[dni], rel=cfg.get("DREL", REL), dl=cfg.get("DDL", DL) if qd + cfg.get("DDL", DL) <= nq else None); dni += 1
            assert ci == len(chain) and dni == len(td) and hi == len(hbt) and deferred is None and not mq
            if MOE == "vpu":
                y = jnp.concatenate([moe[("d", c0)] for c0 in range(0, D // 128, DCOL)], axis=1)
            else:
                y = ymx
            y = rbf(rbf(y) * sel["gate"])
            rows2 = jnp.where(sel["msk"], sel["rows"] + y, sel["rows"])
            xn_buf[pl.ds(sel["g0"], 16), :] = rows2.astype(bf16)

        with scope(cfg, "stD"):
            o_cp = []
            for n in range(NOUT):
                n0 = n * ON
                parts = DTAIL if n == NOUT - 1 else 1
                RB = S // parts
                for pp in range(parts):
                    r0 = pp * RB
                    acc = st.dot(o_buf[pl.ds(r0, RB), :], m_buf[:, pl.ds(n0, ON)], nk=NK, tie_row=min(cfg.get("DTIE", 1024), RB // 2))
                    res = xbuf[pl.ds(r0, RB), pl.ds(n0, ON)].astype(f32) + xn_buf[pl.ds(r0, RB), pl.ds(n0, ON)].astype(f32)
                    xbuf[pl.ds(r0, RB), pl.ds(n0, ON)] = (acc + res).astype(bf16)
                    c = pltpu.make_async_copy(xbuf.at[pl.ds(r0, RB), pl.ds(n0, ON)], out_hbm.at[pl.ds(r0, RB), pl.ds(n0, ON)], out_sems.at[len(o_cp)])
                    c.start()
                    o_cp.append(c)
            for c in o_cp:
                c.wait()

    return kernel, len(XP) + 12, NOUT + DTAIL - 1


def build(cfg=None):
    cfg = cfg or {}
    kernel, nin, nout = make_kernel(cfg)
    anyspec = pl.BlockSpec(memory_space=pl.ANY)
    scratch = [
        pltpu.VMEM((S, D), bf16),
        pltpu.VMEM((S, D), bf16),
        pltpu.VMEM((D, S), bf16),
        pltpu.VMEM((S, D), bf16),
        pltpu.VMEM((D, D), bf16),
        pltpu.VMEM((D, D), bf16),
        pltpu.VMEM((D, D), bf16),
        pltpu.VMEM((D, D), bf16),
        pltpu.VMEM((8, 128), bf16),
        pltpu.VMEM((D, F), bf16),
        pltpu.VMEM((D, F), bf16),
        pltpu.VMEM((F, D), bf16),
        pltpu.VMEM((D, D), bf16),
        pltpu.VMEM((D, D), bf16),
        pltpu.VMEM((D, D), bf16),
        pltpu.VMEM((D, 128), f32),
        pltpu.VMEM((D, 128), f32),
        pltpu.VMEM((F, 128), f32),
        pltpu.VMEM((16, 128), bf16),
        pltpu.SemaphoreType.DMA((nin,)),
        pltpu.SemaphoreType.DMA((nout,)),
    ]
    call = pl.pallas_call(
        kernel,
        out_shape=jax.ShapeDtypeStruct((S, D), bf16),
        in_specs=[anyspec] * 7,
        out_specs=anyspec,
        scratch_shapes=scratch,
        compiler_params=pltpu.CompilerParams(vmem_limit_bytes=cfg.get("VMEM", 110) * 2**20),
        interpret=cfg.get("INTERPRET", False),
    )

    def fn(A_x, A_wqkv, A_wo, B_x, B_w_r, B_w_gate, B_w_up, B_w_down):
        out = call(A_x.reshape(S, D), A_wqkv, A_wo, B_w_r.reshape(8, 128), B_w_gate, B_w_up, B_w_down)
        return out.reshape(1, S, D)

    return fn


_CFG = dict(CHSPLIT=2,CHN=9,DROWS=256,Q1=2,POSTMIX=False,DREL=2,LR=32,LNSPAN=6,PREREL=2,MREL=2,NK=8,DDL=3,PREDL=3)


@jax.jit
def pallas_parallel_sum__linear_attn_block__moe_arch_mod__prompt_kernel(
    A_x: jax.Array,
    A_wqkv: jax.Array,
    A_wo: jax.Array,
    B_x: jax.Array,
    B_w_r: jax.Array,
    B_w_gate: jax.Array,
    B_w_up: jax.Array,
    B_w_down: jax.Array,
):
    return build(_CFG)(A_x, A_wqkv, A_wo, B_x, B_w_r, B_w_gate, B_w_up, B_w_down)
```

```python
import contextlib
import jax
import jax.numpy as jnp
import numpy as np
from jax import lax
from jax.experimental import pallas as pl
from jax.experimental.pallas import tpu as pltpu

S, D, F, H, DH = 2048, 1024, 3584, 32, 32
f32, bf16, i32, u32 = jnp.float32, jnp.bfloat16, jnp.int32, jnp.uint32

NN = (((1,), (0,)), ((), ()))
NT = (((1,), (1,)), ((), ()))
EPS_BF16 = np.float32(1.0013580322265625e-05)


def mm(a, b, dims=NN):
    return lax.dot_general(a, b, dims, preferred_element_type=f32)


def rbf(v):
    return v.astype(bf16).astype(f32)


def phi(t):
    return jnp.where(t > 0, t + 1.0, jnp.exp(t)) + 1e-6


def bits(v):
    return pltpu.bitcast(v, u32)


def orall(vs):
    f = vs[0]
    for o in vs[1:]:
        f = f | o
    return f


def scope(cfg, name):
    return jax.named_scope(name) if cfg.get("SCOPES") else contextlib.nullcontext()


class Stream:
    def __init__(self, enable=True):
        self.Z = None
        self.i = 0
        self.res = {}
        self.pend = {}
        self.enable = enable
        self.bar = 0

    def tie(self, target, src_bits):
        tb = pltpu.bitcast(target, u32)
        return pltpu.bitcast(tb | (src_bits & self.Z), target.dtype)

    def dot(self, lhs, rhs, dims=NN, nk=4, tie_row=0):
        fl = self.pend.pop(self.i, None)
        if fl and self.enable and self.Z is not None:
            f = orall(fl)
            K = lhs.shape[1]
            nk = min(nk, K // 128)
            r = tie_row
            parts = [self.tie(lhs[r:r + 16, j * 128:(j + 1) * 128], f) for j in range(nk)]
            if nk * 128 < K:
                parts.append(lhs[r:r + 16, nk * 128:])
            top = jnp.concatenate(parts, axis=1) if len(parts) > 1 else parts[0]
            lhs = jnp.concatenate(([lhs[:r]] if r else []) + [top, lhs[r + 16:]], axis=0)
        p = mm(lhs, rhs, dims)
        m = p.shape[0]
        self.res[self.i] = p[m - 8:m, 0:128]
        self.i += 1
        return p

    def barrier(self):
        self.res = {}
        self.bar = self.i
        for k in [k for k in self.pend if k <= self.i]:
            pass

    def side(self, task, rel=1, dl=2):
        di = self.i - 1
        relbits = None
        if rel is not None and self.enable and self.Z is not None:
            relv = self.res.get(di - rel)
            if relv is not None:
                relbits = bits(relv)
        f = task(relbits)
        if f is not None and dl is not None:
            self.pend.setdefault(di + dl, []).append(f)

    def gate(self, v, relbits):
        if relbits is None:
            return v
        if v.shape == (8, 128):
            return self.tie(v, relbits)
        top = self.tie(v[0:8, 0:128], relbits)
        row = top if v.shape[1] == 128 else jnp.concatenate([top, v[0:8, 128:]], axis=1)
        return row if v.shape[0] == 8 else jnp.concatenate([row, v[8:]], axis=0)


def gate_all(st, v, relbits):
    if relbits is None:
        return v
    rows = []
    for i in range(v.shape[0] // 8):
        cols = [st.tie(v[i * 8:(i + 1) * 8, j * 128:(j + 1) * 128], relbits) for j in range(v.shape[1] // 128)]
        rows.append(jnp.concatenate(cols, axis=1) if len(cols) > 1 else cols[0])
    return jnp.concatenate(rows, axis=0) if len(rows) > 1 else rows[0]


def spread(ntasks, first, last):
    n = last - first
    out, done = {}, 0
    for s in range(n):
        upto = ntasks * (s + 1) // n
        out[first + s] = upto - done
        done = upto
    return out


def tile_bits_bf16(v):
    a, b = v.shape[0] // 128, v.shape[1] // 128
    return orall([bits(v[i * 128 + 112:(i + 1) * 128, j * 128:(j + 1) * 128]) for i in range(a) for j in range(b)])


def tile_bits_f32(v):
    a, b = v.shape[0] // 128, v.shape[1] // 128
    return orall([bits(v[i * 128 + 120:(i + 1) * 128, j * 128:(j + 1) * 128]) for i in range(a) for j in range(b)])


def make_kernel(cfg):
    LR = cfg.get("LR", 16)
    KM, KN = cfg.get("KM", 256), cfg.get("KN", 256)
    GK = cfg.get("GK", 512)
    GN = cfg.get("GN", 128)
    QT = cfg.get("QT", 128)
    ON = cfg.get("ON", 128)
    MOE = cfg.get("MOE", "vpu")
    MCOL, MROWS = cfg.get("MCOL", 7), cfg.get("MROWS", 256)
    DCOL, DROWS = cfg.get("DCOL", 8), cfg.get("DROWS", 256)
    G1 = cfg.get("G1", 11)
    Q1 = cfg.get("Q1", 3)
    REL, DL = cfg.get("REL", 1), cfg.get("DL", 2)
    NK = cfg.get("NK", 4)
    RR = cfg.get("RR", 64)
    NOUT = D // ON
    DTAIL = cfg.get("DTAIL", 4)
    XP = cfg["XP"]

    def kernel(x_hbm, wqkv_hbm, wo_hbm, wr_hbm, wg_hbm, wu_hbm, wd_hbm, out_hbm,
               xbuf, xn_buf, pkT_buf, o_buf, wq_buf, wk_buf, wv_buf, wo_buf, wr_buf,
               wg_buf, wu_buf, wd_buf, wqT_buf, g_buf, m_buf, zb_buf, xb_buf, hb_buf, z2_buf, in_sems, out_sems):
        sem = iter(range(64))

        def cp(src, dst):
            return pltpu.make_async_copy(src, dst, in_sems.at[next(sem)])

        xs = [0]
        for n in XP:
            xs.append(xs[-1] + n)
        assert xs[-1] == S
        names = {"x%d" % i: cp(x_hbm.at[pl.ds(xs[i], XP[i]), :], xbuf.at[pl.ds(xs[i], XP[i]), :]) for i in range(len(XP))}
        names["z"] = cp(x_hbm.at[pl.ds(0, 16), pl.ds(0, 128)], z2_buf)
        names["wr"] = cp(wr_hbm, wr_buf)
        for j, (c0, nc) in enumerate(cfg.get("QP", [(0, 256), (256, 256), (512, 256), (768, 256)])):
            names["q%d" % j] = cp(wqkv_hbm.at[:, pl.ds(D + c0, nc)], wk_buf.at[:, pl.ds(c0, nc)])
        names["wq"] = cp(wqkv_hbm.at[:, pl.ds(0, D)], wq_buf)
        names["wv"] = cp(wqkv_hbm.at[:, pl.ds(2 * D, D)], wv_buf)
        names["wo"] = cp(wo_hbm, wo_buf)
        names["wg"] = cp(wg_hbm, wg_buf)
        names["wu"] = cp(wu_hbm, wu_buf)
        names["wd"] = cp(wd_hbm, wd_buf)
        order = cfg["ORDER"].split()
        assert sorted(order) == sorted(names)
        for nm in order:
            names[nm].start()

        st = Stream(cfg.get("TIE", True))

        def wait(lst):
            for nm in lst.split():
                with scope(cfg, "w_" + nm):
                    names[nm].wait()
            st.barrier()

        def ln_task(r0):
            def task(relbits):
                x = st.gate(xbuf[pl.ds(r0, LR), :].astype(f32), relbits)
                mean = jnp.sum(x, axis=1, keepdims=True) * (1.0 / D)
                d = x - mean
                var = jnp.sum(d * d, axis=1, keepdims=True) * (1.0 / D)
                t3 = rbf(jnp.sqrt(rbf(rbf(var) + EPS_BF16)))
                xn = d * (1.0 / t3)
                xn_buf[pl.ds(r0, LR), :] = xn.astype(bf16)
                return orall([bits(xn[g * 8:(g + 1) * 8, D - 128:D]) for g in range(LR // 8)])
            return task

        def ln_rows(a, b):
            for r0 in range(a, b, LR):
                ln_task(r0)(None)

        zacc = {}
        with scope(cfg, "stA"):
            ncb = D // KN
            U = cfg["UNITS"]
            WA = cfg["WA"]
            cover = np.zeros((S // 128, ncb), int)
            for (r0, nr, cb) in U:
                cover[r0 // 128:(r0 + nr) // 128, cb] += 1
            assert (cover == 1).all()
            wait(cfg["W0"])
            ln_rows(0, cfg["LN0"])
            st.Z = bits(z2_buf[...]) ^ bits(xbuf[0:16, 0:128])
            slots = {}
            for (a, b, u_first, u_last) in cfg["LNS"]:
                tl = [ln_task(r) for r in range(a, b, LR)]
                u_need = min(ui for ui, (r0, nr, cb) in enumerate(U) if r0 < b and r0 + nr > a)
                assert u_first < u_last <= u_need, (a, b, u_first, u_last, u_need)
                cnt = spread(len(tl), u_first, u_last)
                ti = 0
                for j in range(u_first, u_last):
                    for _ in range(cnt[j]):
                        slots.setdefault(j, []).append((tl[ti], u_need)); ti += 1

            def k_epilogue(r0, nr, cb, p):
                def task(relbits):
                    pk = phi(p)
                    zp = jnp.sum(pk.reshape(nr // 8, 8, KN), axis=0)
                    zacc[cb] = zp if cb not in zacc else zacc[cb] + zp
                    pt = pk.astype(bf16).T
                    pkT_buf[pl.ds(cb * KN, KN), pl.ds(r0, nr)] = pt
                    return tile_bits_bf16(pt)
                return task

            deferred = None
            for ui, (r0, nr, cb) in enumerate(U):
                if ui in WA:
                    wait(WA[ui])
                p = st.dot(xn_buf[pl.ds(r0, nr), :], wk_buf[:, pl.ds(cb * KN, KN)], nk=NK)
                nxtw = min([w for w in WA if w > ui] + [10 ** 9])
                if deferred is not None:
                    DD = cfg.get("DEFDL", 2)
                    st.side(deferred, rel=None, dl=DD if ui + DD < nxtw else None); deferred = None
                ep = k_epilogue(r0, nr, cb, p)
                if ui + 1 == nxtw and cfg.get("DEFER", True) and ui >= cfg.get("DEFER0", 0):
                    deferred = ep
                else:
                    KE = cfg.get("KEDL", DL)
                    st.side(ep, rel=None, dl=KE if ui + KE < nxtw else None)
                for (t, u_need) in slots.get(ui, []):
                    dl = min(cfg.get("LNDL", DL), u_need - ui)
                    st.side(t, rel=cfg.get("LNREL", REL), dl=dl if ui + dl < nxtw else None)
            assert deferred is None

        rstate = {}

        def router_task(r0):
            def task(relbits):
                if "wr" not in rstate:
                    w8 = wr_buf[...].astype(f32)
                    rstate["wr"] = jnp.concatenate([w8[j:j + 1, :] for j in range(8)], axis=1)
                    rstate["best"] = jnp.full((RR, 1), -jnp.inf, f32)
                    rstate["bidx"] = jnp.zeros((RR, 1), f32)
                    rstate["iota"] = lax.broadcasted_iota(i32, (RR, 1), 0).astype(f32)
                xn = st.gate(xn_buf[pl.ds(r0, RR), :].astype(f32), relbits)
                pr = xn * rstate["wr"]
                sp = pr[:, 0:128]
                for j in range(1, D // 128):
                    sp = sp + pr[:, j * 128:(j + 1) * 128]
                r = rbf(jnp.sum(sp, axis=1, keepdims=True))
                c = r > rstate["best"]
                rstate["best"] = jnp.where(c, r, rstate["best"])
                rstate["bidx"] = jnp.where(c, rstate["iota"] + np.float32(r0), rstate["bidx"])
                return orall([bits(sp[g * 8:(g + 1) * 8]) for g in range(RR // 8)])
            return task

        sel = {}

        def router_final(relbits):
            best, bidx = rstate["best"], rstate["bidx"]
            m = jnp.max(best)
            cand = jnp.where(best == m, bidx, np.float32(2 * S))
            idx = jnp.clip(jnp.min(cand).astype(i32), 0, S - 1)
            g0 = pl.multiple_of((idx // 16) * 16, 16)
            rows = xn_buf[pl.ds(g0, 16), :].astype(f32)
            msk = lax.broadcasted_iota(i32, (16, D), 0) == (idx - g0)
            xrow = jnp.sum(jnp.where(msk, rows, 0.0), axis=0, keepdims=True)
            rsel = rbf(jnp.sum(xrow * rstate["wr"], axis=1, keepdims=True))
            sel.update(idx=idx, g0=g0, rows=rows, msk=msk, xrow=xrow, gate=rbf(1.0 / (1.0 + jnp.exp(-rsel))))
            if MOE == "vpu":
                xb = jnp.broadcast_to(xrow, (128, D)).T
                xb_buf[...] = xb
                return tile_bits_f32(xb)
            return None

        def zb_task(relbits):
            z = jnp.concatenate([jnp.sum(zacc[cb], axis=0, keepdims=True) for cb in range(D // KN)], axis=1)
            z = st.gate(jnp.broadcast_to(z, (8, D)), relbits)
            zb = jnp.broadcast_to(z[0:1], (128, D)).T
            zb_buf[...] = zb
            return tile_bits_f32(zb)

        def wqT_task(j):
            def task(relbits):
                w = wq_buf[:, pl.ds(j * 128, 128)]
                if relbits is not None:
                    w = jnp.concatenate([st.tie(w[0:16], relbits), w[16:]], axis=0)
                wt = w.T
                wqT_buf[pl.ds(j * 128, 128), :] = wt
                return tile_bits_bf16(wt)
            return task

        moe = {}

        def mv_tasks(w_ref, b_ref, K, ncolt, key, ncol, rows):
            ts = []
            for c0 in range(0, ncolt, ncol):
                state = {}
                for k0 in range(0, K, rows):
                    def task(relbits, c0=c0, k0=k0, state=state):
                        acc = state.get("acc")
                        for k in range(k0, k0 + rows, 16):
                            w = w_ref[k:k + 16, c0 * 128:(c0 + ncol) * 128].astype(f32)
                            xb = b_ref[k:k + 16, :]
                            if (k - k0) % cfg.get("MGATE", 10 ** 6) == 0:
                                xb = gate_all(st, xb, relbits) if cfg.get("MGATEALL", False) else st.gate(xb, relbits)
                            p = jnp.concatenate([w[:, j * 128:(j + 1) * 128] * xb for j in range(ncol)], axis=1)
                            p = p[0:8] + p[8:16]
                            acc = p if acc is None else acc + p
                        state["acc"] = acc
                        if k0 + rows == K:
                            moe[(key, c0)] = jnp.sum(acc, axis=0, keepdims=True)
                        return orall([bits(acc[:, j * 128:(j + 1) * 128]) for j in range(ncol)])
                    ts.append(task)
            return ts

        def hb_task(c0):
            def task(relbits):
                g = gate_all(st, jnp.broadcast_to(moe[("g", c0)], (8, MCOL * 128)), relbits)[0:1]
                u = moe[("u", c0)]
                g = rbf(g)
                h = rbf(rbf(g * (1.0 / (1.0 + jnp.exp(-g)))) * rbf(u))
                hb = jnp.broadcast_to(h, (128, MCOL * 128)).T
                hb_buf[pl.ds(c0 * 128, MCOL * 128), :] = hb
                return tile_bits_f32(hb)
            return task

        with scope(cfg, "stG"):
            nsub = (D // GN) * (S // GK)
            wqt = [wqT_task(j) for j in range(D // 128)]
            pre = [router_task(r) for r in range(0, S, RR)] + [router_final, zb_task] + (wqt if cfg.get("WQT_PRE", True) else [])
            post = []
            nhb_g = 0
            if MOE == "vpu":
                tg = mv_tasks(wg_buf, xb_buf, D, F // 128, "g", MCOL, MROWS)
                tu = mv_tasks(wu_buf, xb_buf, D, F // 128, "u", MCOL, MROWS)
                per = D // MROWS
                ngrp = len(tg) // per
                if cfg.get("POSTMIX", True):
                    HBLAG = cfg.get("HBLAG", 2)
                    hbq = []
                    for gi in range(ngrp):
                        for j, t in enumerate(tg[gi * per:(gi + 1) * per] + tu[gi * per:(gi + 1) * per]):
                            post.append(t)
                            if j == HBLAG - 1 and hbq:
                                post.append(hbq.pop(0)); nhb_g += 1
                        hbq.append(hb_task(gi * MCOL))
                else:
                    post = tg + tu
            if not cfg.get("WQT_PRE", True):
                post = wqt + post
            c_pre = spread(len(pre), 0, G1 - 1)
            c_post = spread(len(post), G1, nsub - cfg.get("GEND", 1))
            pi = qi = di = 0
            for n in range(D // GN):
                acc = None
                for kc in range(S // GK):
                    if di == G1:
                        wait(cfg.get("WG1", "wg wu"))
                    p = st.dot(pkT_buf[:, pl.ds(kc * GK, GK)], xn_buf[pl.ds(kc * GK, GK), pl.ds(n * GN, GN)], nk=NK)
                    acc = p if acc is None else acc + p
                    if kc == S // GK - 1:
                        g_buf[:, pl.ds(n * GN, GN)] = acc.astype(bf16)
                    for _ in range(c_pre.get(di, 0)):
                        PD = cfg.get("PREDL", DL)
                        st.side(pre[pi], rel=cfg.get("PREREL", REL), dl=PD if di + PD < G1 else None); pi += 1
                    for _ in range(c_post.get(di, 0)):
                        st.side(post[qi], rel=cfg.get("MREL", REL), dl=cfg.get("MDL", DL)); qi += 1
                    di += 1
            assert pi == len(pre) and qi == len(post)

        with scope(cfg, "stQ"):
            td = mv_tasks(wd_buf, hb_buf, F, D // 128, "d", DCOL, DROWS) if MOE == "vpu" else []
            rr = lax.broadcasted_iota(i32, (128, 128), 0) // DH
            cc = lax.broadcasted_iota(i32, (128, 128), 1) // DH
            bd = rr == cc

            def chain_task(c):
                def task(relbits):
                    kv = mm(g_buf[pl.ds(c * 128, 128), :], wv_buf[:, pl.ds(c * 128, 128)])
                    kv = jnp.where(bd, kv, 0.0).astype(bf16)
                    m_buf[pl.ds(c * 128, 128), :] = mm(kv, wo_buf[pl.ds(c * 128, 128), :]).astype(bf16)
                    return None
                return task

            kvs = {}

            def kv_task(c):
                def task(relbits):
                    kv = mm(g_buf[pl.ds(c * 128, 128), :], wv_buf[:, pl.ds(c * 128, 128)])
                    kvs[c] = jnp.where(bd, kv, 0.0).astype(bf16)
                    return None
                return task

            def m_task(c):
                def task(relbits):
                    m_buf[pl.ds(c * 128, 128), :] = mm(kvs[c], wo_buf[pl.ds(c * 128, 128), :]).astype(bf16)
                    return None
                return task

            def q_epilogue(t0, q):
                def task(relbits):
                    pq = phi(q)
                    zb = zb_buf[...]
                    tz = jnp.concatenate([pq[:, j * 128:(j + 1) * 128] * zb for j in range(QT // 128)], axis=1) if QT > 128 else pq * zb
                    den = jnp.sum(tz.reshape(H, DH, QT), axis=1, keepdims=True) + 1e-6
                    o = (pq.reshape(H, DH, QT) * (1.0 / den)).reshape(D, QT)
                    ot = o.astype(bf16).T
                    o_buf[pl.ds(t0, QT), :] = ot
                    return tile_bits_bf16(ot)
                return task

            nq = S // QT
            hbt = [hb_task(c0) for c0 in range(0, F // 128, MCOL)][nhb_g:] if MOE == "vpu" else []
            c_hb = spread(len(hbt), cfg.get("HB0", 0), max(cfg.get("HB0", 0) + 1, Q1 - 1))
            chain = [chain_task(c) for c in range(D // 128)]
            c_chain = spread(len(chain), Q1 + cfg.get("CH0", 0), min(nq, Q1 + cfg.get("CH0", 0) + cfg.get("CHN", 8)))
            CHS = cfg.get("CHSPLIT", 0)
            mq = {}
            c_down = spread(len(td), Q1, nq - cfg.get("DEND", 1))
            ci = dni = hi = 0
            deferred = None
            for qd in range(nq):
                t0 = qd * QT
                if qd == Q1:
                    wait("wv wo wd")
                    if MOE != "vpu":
                        x16 = jnp.broadcast_to(sel["xrow"], (16, D)).astype(bf16)
                        g = rbf(mm(x16, wg_buf[...]))
                        u = rbf(mm(x16, wu_buf[...]))
                        h = rbf(g * (1.0 / (1.0 + jnp.exp(-g)))) * u
                        ymx = mm(h.astype(bf16), wd_buf[...])[0:1, :]
                q = st.dot(wqT_buf[...], xn_buf[pl.ds(t0, QT), :], NT, nk=NK)
                if deferred is not None:
                    st.side(deferred, rel=None, dl=cfg.get("DEFDL", 2)); deferred = None
                ep = q_epilogue(t0, q)
                if qd + 1 == Q1 and cfg.get("DEFER", True):
                    deferred = ep
                else:
                    QE = cfg.get("QEDL", DL)
                    st.side(ep, rel=None, dl=QE if (not (qd < Q1 <= qd + QE) and qd + QE < nq + cfg.get("QTAIL", 2)) else None)
                for _ in range(c_hb.get(qd, 0)):
                    st.side(hbt[hi], rel=REL, dl=DL if qd + DL < Q1 else None); hi += 1
                for c in mq.pop(qd, []):
                    st.side(m_task(c), rel=None, dl=None)
                for _ in range(c_chain.get(qd, 0)):
                    if CHS:
                        st.side(kv_task(ci), rel=None, dl=None); mq.setdefault(min(qd + CHS, nq - 1), []).append(ci)
                    else:
                        st.side(chain[ci], rel=None, dl=None)
                    ci += 1
                for _ in range(c_down.get(qd, 0)):
                    st.side(td[dni], rel=cfg.get("DREL", REL), dl=cfg.get("DDL", DL) if qd + cfg.get("DDL", DL) <= nq else None); dni += 1
            assert ci == len(chain) and dni == len(td) and hi == len(hbt) and deferred is None and not mq
            if MOE == "vpu":
                y = jnp.concatenate([moe[("d", c0)] for c0 in range(0, D // 128, DCOL)], axis=1)
            else:
                y = ymx
            y = rbf(rbf(y) * sel["gate"])
            rows2 = jnp.where(sel["msk"], sel["rows"] + y, sel["rows"])
            xn_buf[pl.ds(sel["g0"], 16), :] = rows2.astype(bf16)

        with scope(cfg, "stD"):
            o_cp = []
            for n in range(NOUT):
                n0 = n * ON
                parts = DTAIL if n == NOUT - 1 else 1
                RB = S // parts
                for pp in range(parts):
                    r0 = pp * RB
                    acc = st.dot(o_buf[pl.ds(r0, RB), :], m_buf[:, pl.ds(n0, ON)], nk=NK, tie_row=min(cfg.get("DTIE", 1024), RB // 2))
                    res = xbuf[pl.ds(r0, RB), pl.ds(n0, ON)].astype(f32) + xn_buf[pl.ds(r0, RB), pl.ds(n0, ON)].astype(f32)
                    xbuf[pl.ds(r0, RB), pl.ds(n0, ON)] = (acc + res).astype(bf16)
                    c = pltpu.make_async_copy(xbuf.at[pl.ds(r0, RB), pl.ds(n0, ON)], out_hbm.at[pl.ds(r0, RB), pl.ds(n0, ON)], out_sems.at[len(o_cp)])
                    c.start()
                    o_cp.append(c)
            for c in o_cp:
                c.wait()

    return kernel, len(XP) + 8 + len(cfg.get('QP', [0] * 4)), NOUT + DTAIL - 1


def _k_units(rows):
    return [(r0, 256, cb) for r0 in rows for cb in range(4)]


START_A = dict(
    XP=[256, 256, 256, 512, 768], ORDER="x0 x1 z q0 q1 x2 q2 q3 x3 wr x4 wq wg wu wv wo wd", W0="x0 x1 z", LN0=512,
    UNITS=[(0, 256, 0), (256, 256, 0), (0, 256, 1), (256, 256, 1), (0, 256, 2), (256, 256, 2), (512, 256, 0), (512, 256, 1), (512, 256, 2),
           (0, 256, 3), (256, 256, 3), (512, 256, 3)] + _k_units(range(768, 2048, 256)),
    WA={0: "q0", 2: "q1", 4: "q2 x2", 9: "q3 x3", 16: "x4 wr wq"},
    LNS=[(512, 768, 4, 6), (768, 1024, 9, 12), (1024, 1280, 10, 16), (1280, 1536, 16, 20), (1536, 1792, 18, 24), (1792, 2048, 22, 28)])
START_B = dict(
    XP=[256, 128, 128, 256, 512, 768], ORDER="q0 z x0 x1 x2 q1 q2 x3 q3 x4 wr x5 wq wg wu wv wo wd", W0="q0 z x0", LN0=256,
    UNITS=[(0, 256, 0), (256, 128, 0), (384, 128, 0), (0, 256, 1), (256, 256, 1), (0, 256, 2), (256, 256, 2), (512, 256, 0), (512, 256, 1), (512, 256, 2),
           (0, 256, 3), (256, 256, 3), (512, 256, 3)] + _k_units(range(768, 2048, 256)),
    WA={0: "x1", 1: "x2", 3: "q1", 5: "q2 x3", 10: "q3 x4", 17: "x5 wr wq"},
    LNS=[(256, 384, 0, 1), (384, 512, 1, 2), (512, 768, 5, 7), (768, 1024, 10, 13), (1024, 1280, 11, 17), (1280, 1536, 17, 21), (1536, 1792, 19, 25), (1792, 2048, 23, 29)])


def build(cfg=None):
    cfg = dict(cfg or {})
    for k, v in (START_B if cfg.get("START", "B") == "B" else START_A).items():
        cfg.setdefault(k, v)
    kernel, nin, nout = make_kernel(cfg)
    anyspec = pl.BlockSpec(memory_space=pl.ANY)
    scratch = [
        pltpu.VMEM((S, D), bf16),
        pltpu.VMEM((S, D), bf16),
        pltpu.VMEM((D, S), bf16),
        pltpu.VMEM((S, D), bf16),
        pltpu.VMEM((D, D), bf16),
        pltpu.VMEM((D, D), bf16),
        pltpu.VMEM((D, D), bf16),
        pltpu.VMEM((D, D), bf16),
        pltpu.VMEM((8, 128), bf16),
        pltpu.VMEM((D, F), bf16),
        pltpu.VMEM((D, F), bf16),
        pltpu.VMEM((F, D), bf16),
        pltpu.VMEM((D, D), bf16),
        pltpu.VMEM((D, D), bf16),
        pltpu.VMEM((D, D), bf16),
        pltpu.VMEM((D, 128), f32),
        pltpu.VMEM((D, 128), f32),
        pltpu.VMEM((F, 128), f32),
        pltpu.VMEM((16, 128), bf16),
        pltpu.SemaphoreType.DMA((nin,)),
        pltpu.SemaphoreType.DMA((nout,)),
    ]
    call = pl.pallas_call(
        kernel,
        out_shape=jax.ShapeDtypeStruct((S, D), bf16),
        in_specs=[anyspec] * 7,
        out_specs=anyspec,
        scratch_shapes=scratch,
        compiler_params=pltpu.CompilerParams(vmem_limit_bytes=cfg.get("VMEM", 110) * 2**20),
        interpret=cfg.get("INTERPRET", False),
    )

    def fn(A_x, A_wqkv, A_wo, B_x, B_w_r, B_w_gate, B_w_up, B_w_down):
        out = call(A_x.reshape(S, D), A_wqkv, A_wo, B_w_r.reshape(8, 128), B_w_gate, B_w_up, B_w_down)
        return out.reshape(1, S, D)

    return fn


_CFG = {'CHSPLIT': 2, 'CHN': 9, 'DROWS': 256, 'Q1': 2, 'POSTMIX': False, 'DREL': 2, 'PREREL': 3, 'MREL': 2, 'NK': 8, 'DDL': 3, 'PREDL': 3, 'LR': 16, 'XP': [256, 128, 128, 256, 512, 768], 'ORDER': 'x0 z x1 q0 x2 q1 q2 x3 q3 x4 wr x5 wq wg wu wv wo wd', 'W0': 'x0 z x1', 'LN0': 384, 'UNITS': [(0, 256, 0), (256, 128, 0), (384, 128, 0), (0, 256, 1), (256, 256, 1), (0, 256, 2), (256, 256, 2), (512, 256, 0), (512, 256, 1), (512, 256, 2), (0, 256, 3), (256, 256, 3), (512, 256, 3), (768, 256, 0), (768, 256, 1), (768, 256, 2), (768, 256, 3), (1024, 256, 0), (1024, 256, 1), (1024, 256, 2), (1024, 256, 3), (1280, 256, 0), (1280, 256, 1), (1280, 256, 2), (1280, 256, 3), (1536, 256, 0), (1536, 256, 1), (1536, 256, 2), (1536, 256, 3), (1792, 256, 0), (1792, 256, 1), (1792, 256, 2), (1792, 256, 3)], 'WA': {0: 'q0', 1: 'x2', 3: 'q1', 5: 'q2 x3', 10: 'q3 x4', 17: 'x5 wr wq'}, 'LNS': [(384, 512, 1, 2), (512, 768, 5, 7), (768, 1024, 10, 13), (1024, 1280, 11, 17), (1280, 1536, 17, 21), (1536, 1792, 19, 25), (1792, 2048, 23, 29)]}


@jax.jit
def pallas_parallel_sum__linear_attn_block__moe_arch_mod__prompt_kernel(
    A_x: jax.Array,
    A_wqkv: jax.Array,
    A_wo: jax.Array,
    B_x: jax.Array,
    B_w_r: jax.Array,
    B_w_gate: jax.Array,
    B_w_up: jax.Array,
    B_w_down: jax.Array,
):
    return build(_CFG)(A_x, A_wqkv, A_wo, B_x, B_w_r, B_w_gate, B_w_up, B_w_down)
```

```python
import contextlib
import jax
import jax.numpy as jnp
import numpy as np
from jax import lax
from jax.experimental import pallas as pl
from jax.experimental.pallas import tpu as pltpu

S, D, F, H, DH = 2048, 1024, 3584, 32, 32
f32, bf16, i32, u32 = jnp.float32, jnp.bfloat16, jnp.int32, jnp.uint32

NN = (((1,), (0,)), ((), ()))
NT = (((1,), (1,)), ((), ()))
EPS_BF16 = np.float32(1.0013580322265625e-05)


def mm(a, b, dims=NN):
    return lax.dot_general(a, b, dims, preferred_element_type=f32)


def rbf(v):
    return v.astype(bf16).astype(f32)


def phi(t):
    return jnp.where(t > 0, t + 1.0, jnp.exp(t)) + 1e-6


def bits(v):
    return pltpu.bitcast(v, u32)


def orall(vs):
    f = vs[0]
    for o in vs[1:]:
        f = f | o
    return f


def scope(cfg, name):
    return jax.named_scope(name) if cfg.get("SCOPES") else contextlib.nullcontext()


class Stream:
    def __init__(self, enable=True):
        self.Z = None
        self.i = 0
        self.res = {}
        self.pend = {}
        self.enable = enable
        self.bar = 0

    def tie(self, target, src_bits):
        tb = pltpu.bitcast(target, u32)
        return pltpu.bitcast(tb | (src_bits & self.Z), target.dtype)

    def dot(self, lhs, rhs, dims=NN, nk=4, tie_row=0):
        fl = self.pend.pop(self.i, None)
        if fl and self.enable and self.Z is not None:
            f = orall(fl)
            K = lhs.shape[1]
            nk = min(nk, K // 128)
            r = tie_row
            parts = [self.tie(lhs[r:r + 16, j * 128:(j + 1) * 128], f) for j in range(nk)]
            if nk * 128 < K:
                parts.append(lhs[r:r + 16, nk * 128:])
            top = jnp.concatenate(parts, axis=1) if len(parts) > 1 else parts[0]
            lhs = jnp.concatenate(([lhs[:r]] if r else []) + [top, lhs[r + 16:]], axis=0)
        p = mm(lhs, rhs, dims)
        m = p.shape[0]
        self.res[self.i] = p[m - 8:m, 0:128]
        self.i += 1
        return p

    def barrier(self):
        self.res = {}
        self.bar = self.i
        for k in [k for k in self.pend if k <= self.i]:
            pass

    def side(self, task, rel=1, dl=2):
        di = self.i - 1
        relbits = None
        if rel is not None and self.enable and self.Z is not None:
            relv = self.res.get(di - rel)
            if relv is not None:
                relbits = bits(relv)
        f = task(relbits)
        if f is not None and dl is not None:
            self.pend.setdefault(di + dl, []).append(f)

    def gate(self, v, relbits):
        if relbits is None:
            return v
        if v.shape == (8, 128):
            return self.tie(v, relbits)
        top = self.tie(v[0:8, 0:128], relbits)
        row = top if v.shape[1] == 128 else jnp.concatenate([top, v[0:8, 128:]], axis=1)
        return row if v.shape[0] == 8 else jnp.concatenate([row, v[8:]], axis=0)


def gate_all(st, v, relbits):
    if relbits is None:
        return v
    rows = []
    for i in range(v.shape[0] // 8):
        cols = [st.tie(v[i * 8:(i + 1) * 8, j * 128:(j + 1) * 128], relbits) for j in range(v.shape[1] // 128)]
        rows.append(jnp.concatenate(cols, axis=1) if len(cols) > 1 else cols[0])
    return jnp.concatenate(rows, axis=0) if len(rows) > 1 else rows[0]


def spread(ntasks, first, last):
    n = last - first
    out, done = {}, 0
    for s in range(n):
        upto = ntasks * (s + 1) // n
        out[first + s] = upto - done
        done = upto
    return out


def tile_bits_bf16(v):
    a, b = v.shape[0] // 128, v.shape[1] // 128
    return orall([bits(v[i * 128 + 112:(i + 1) * 128, j * 128:(j + 1) * 128]) for i in range(a) for j in range(b)])


def tile_bits_f32(v):
    a, b = v.shape[0] // 128, v.shape[1] // 128
    return orall([bits(v[i * 128 + 120:(i + 1) * 128, j * 128:(j + 1) * 128]) for i in range(a) for j in range(b)])


def make_kernel(cfg):
    LR = cfg.get("LR", 16)
    KM, KN = cfg.get("KM", 256), cfg.get("KN", 256)
    GK = cfg.get("GK", 512)
    GN = cfg.get("GN", 128)
    QT = cfg.get("QT", 128)
    ON = cfg.get("ON", 128)
    MOE = cfg.get("MOE", "vpu")
    MCOL, MROWS = cfg.get("MCOL", 7), cfg.get("MROWS", 256)
    DCOL, DROWS = cfg.get("DCOL", 8), cfg.get("DROWS", 256)
    G1 = cfg.get("G1", 11)
    Q1 = cfg.get("Q1", 3)
    REL, DL = cfg.get("REL", 1), cfg.get("DL", 2)
    NK = cfg.get("NK", 4)
    RR = cfg.get("RR", 64)
    NOUT = D // ON
    DTAIL = cfg.get("DTAIL", 4)
    XP = cfg["XP"]

    def kernel(x_hbm, wqkv_hbm, wo_hbm, wr_hbm, wg_hbm, wu_hbm, wd_hbm, out_hbm,
               xbuf, xn_buf, pkT_buf, o_buf, wq_buf, wk_buf, wv_buf, wo_buf, wr_buf,
               wg_buf, wu_buf, wd_buf, wqT_buf, g_buf, m_buf, zb_buf, xb_buf, hb_buf, z2_buf, sems):
        SEM = cfg["SEM"]

        def cp_named(nm, src, dst):
            return pltpu.make_async_copy(src, dst, sems.at[SEM[nm]])

        xs = [0]
        for n in XP:
            xs.append(xs[-1] + n)
        assert xs[-1] == S
        names = {"x%d" % i: cp_named("x%d" % i, x_hbm.at[pl.ds(xs[i], XP[i]), :], xbuf.at[pl.ds(xs[i], XP[i]), :]) for i in range(len(XP))}
        names["z"] = cp_named("z", x_hbm.at[pl.ds(0, 16), pl.ds(0, 128)], z2_buf)
        names["wr"] = cp_named("wr", wr_hbm, wr_buf)
        for j, (c0, nc) in enumerate(cfg.get("QP", [(0, 256), (256, 256), (512, 256), (768, 256)])):
            names["q%d" % j] = cp_named("q%d" % j, wqkv_hbm.at[:, pl.ds(D + c0, nc)], wk_buf.at[:, pl.ds(c0, nc)])
        names["wq"] = cp_named("wq", wqkv_hbm.at[:, pl.ds(0, D)], wq_buf)
        names["wv"] = cp_named("wv", wqkv_hbm.at[:, pl.ds(2 * D, D)], wv_buf)
        names["wo"] = cp_named("wo", wo_hbm, wo_buf)
        names["wg"] = cp_named("wg", wg_hbm, wg_buf)
        names["wu"] = cp_named("wu", wu_hbm, wu_buf)
        names["wd"] = cp_named("wd", wd_hbm, wd_buf)
        order = cfg["ORDER"].split()
        AFTER = cfg.get("AFTER", {})
        assert sorted(order + [n for v in AFTER.values() for n in v.split()]) == sorted(names)
        for nm in order:
            names[nm].start()

        st = Stream(cfg.get("TIE", True))

        def wait(lst):
            for nm in lst.split():
                with scope(cfg, "w_" + nm):
                    names[nm].wait()
            for nm in AFTER.get(lst, "").split():
                names[nm].start()
            st.barrier()

        def ln_task(r0):
            def task(relbits):
                x = st.gate(xbuf[pl.ds(r0, LR), :].astype(f32), relbits)
                mean = jnp.sum(x, axis=1, keepdims=True) * (1.0 / D)
                d = x - mean
                var = jnp.sum(d * d, axis=1, keepdims=True) * (1.0 / D)
                t3 = rbf(jnp.sqrt(rbf(rbf(var) + EPS_BF16)))
                xn = d * (1.0 / t3)
                xn_buf[pl.ds(r0, LR), :] = xn.astype(bf16)
                return orall([bits(xn[g * 8:(g + 1) * 8, D - 128:D]) for g in range(LR // 8)])
            return task

        def ln_rows(a, b):
            for r0 in range(a, b, LR):
                ln_task(r0)(None)

        zacc = {}
        with scope(cfg, "stA"):
            ncb = D // KN
            U = cfg["UNITS"]
            WA = cfg["WA"]
            cover = np.zeros((S // 128, ncb), int)
            for (r0, nr, cb) in U:
                cover[r0 // 128:(r0 + nr) // 128, cb] += 1
            assert (cover == 1).all()
            wait(cfg["W0"])
            ln_rows(0, cfg["LN0"])
            st.Z = bits(z2_buf[...]) ^ bits(xbuf[0:16, 0:128])
            slots = {}
            for (a, b, u_first, u_last) in cfg["LNS"]:
                tl = [ln_task(r) for r in range(a, b, LR)]
                u_need = min(ui for ui, (r0, nr, cb) in enumerate(U) if r0 < b and r0 + nr > a)
                assert u_first < u_last <= u_need, (a, b, u_first, u_last, u_need)
                cnt = spread(len(tl), u_first, u_last)
                ti = 0
                for j in range(u_first, u_last):
                    for _ in range(cnt[j]):
                        slots.setdefault(j, []).append((tl[ti], u_need)); ti += 1

            def k_epilogue(r0, nr, cb, p):
                def task(relbits):
                    pk = phi(p)
                    zp = jnp.sum(pk.reshape(nr // 8, 8, KN), axis=0)
                    zacc[cb] = zp if cb not in zacc else zacc[cb] + zp
                    pt = pk.astype(bf16).T
                    pkT_buf[pl.ds(cb * KN, KN), pl.ds(r0, nr)] = pt
                    return tile_bits_bf16(pt)
                return task

            deferred = None
            for ui, (r0, nr, cb) in enumerate(U):
                if ui in WA:
                    wait(WA[ui])
                p = st.dot(xn_buf[pl.ds(r0, nr), :], wk_buf[:, pl.ds(cb * KN, KN)], nk=NK)
                nxtw = min([w for w in WA if w > ui] + [10 ** 9])
                if deferred is not None:
                    DD = cfg.get("DEFDLK", 1)
                    st.side(deferred, rel=None, dl=DD if ui + DD < nxtw else None); deferred = None
                ep = k_epilogue(r0, nr, cb, p)
                if ui + 1 == nxtw and cfg.get("DEFER", True) and ui >= cfg.get("DEFER0", 0):
                    deferred = ep
                else:
                    KE = cfg.get("KEDL", DL)
                    st.side(ep, rel=None, dl=KE if ui + KE < nxtw else None)
                for (t, u_need) in slots.get(ui, []):
                    dl = min(cfg.get("LNDL", DL), u_need - ui)
                    st.side(t, rel=cfg.get("LNREL", REL), dl=dl if ui + dl < nxtw else None)
            assert deferred is None

        rstate = {}

        def router_task(r0):
            def task(relbits):
                if "wr" not in rstate:
                    w8 = wr_buf[...].astype(f32)
                    rstate["wr"] = jnp.concatenate([w8[j:j + 1, :] for j in range(8)], axis=1)
                    rstate["best"] = jnp.full((RR, 1), -jnp.inf, f32)
                    rstate["bidx"] = jnp.zeros((RR, 1), f32)
                    rstate["iota"] = lax.broadcasted_iota(i32, (RR, 1), 0).astype(f32)
                xn = st.gate(xn_buf[pl.ds(r0, RR), :].astype(f32), relbits)
                pr = xn * rstate["wr"]
                sp = pr[:, 0:128]
                for j in range(1, D // 128):
                    sp = sp + pr[:, j * 128:(j + 1) * 128]
                r = rbf(jnp.sum(sp, axis=1, keepdims=True))
                c = r > rstate["best"]
                rstate["best"] = jnp.where(c, r, rstate["best"])
                rstate["bidx"] = jnp.where(c, rstate["iota"] + np.float32(r0), rstate["bidx"])
                return orall([bits(sp[g * 8:(g + 1) * 8]) for g in range(RR // 8)])
            return task

        sel = {}

        def router_final(relbits):
            best, bidx = rstate["best"], rstate["bidx"]
            m = jnp.max(best)
            cand = jnp.where(best == m, bidx, np.float32(2 * S))
            idx = jnp.clip(jnp.min(cand).astype(i32), 0, S - 1)
            g0 = pl.multiple_of((idx // 16) * 16, 16)
            rows = xn_buf[pl.ds(g0, 16), :].astype(f32)
            msk = lax.broadcasted_iota(i32, (16, D), 0) == (idx - g0)
            xrow = jnp.sum(jnp.where(msk, rows, 0.0), axis=0, keepdims=True)
            rsel = rbf(jnp.sum(xrow * rstate["wr"], axis=1, keepdims=True))
            sel.update(idx=idx, g0=g0, rows=rows, msk=msk, xrow=xrow, gate=rbf(1.0 / (1.0 + jnp.exp(-rsel))))
            if MOE == "vpu":
                xb = jnp.broadcast_to(xrow, (128, D)).T
                xb_buf[...] = xb
                return tile_bits_f32(xb)
            return None

        def zb_task(relbits):
            z = jnp.concatenate([jnp.sum(zacc[cb], axis=0, keepdims=True) for cb in range(D // KN)], axis=1)
            z = st.gate(jnp.broadcast_to(z, (8, D)), relbits)
            zb = jnp.broadcast_to(z[0:1], (128, D)).T
            zb_buf[...] = zb
            return tile_bits_f32(zb)

        def wqT_task(j):
            def task(relbits):
                w = wq_buf[:, pl.ds(j * 128, 128)]
                if relbits is not None:
                    w = jnp.concatenate([st.tie(w[0:16], relbits), w[16:]], axis=0)
                wt = w.T
                wqT_buf[pl.ds(j * 128, 128), :] = wt
                return tile_bits_bf16(wt)
            return task

        moe = {}

        def mv_tasks(w_ref, b_ref, K, ncolt, key, ncol, rows):
            ts = []
            for c0 in range(0, ncolt, ncol):
                state = {}
                for k0 in range(0, K, rows):
                    def task(relbits, c0=c0, k0=k0, state=state):
                        acc = state.get("acc")
                        for k in range(k0, k0 + rows, 16):
                            w = w_ref[k:k + 16, c0 * 128:(c0 + ncol) * 128].astype(f32)
                            xb = b_ref[k:k + 16, :]
                            if (k - k0) % cfg.get("MGATE", 10 ** 6) == 0:
                                xb = gate_all(st, xb, relbits) if cfg.get("MGATEALL", False) else st.gate(xb, relbits)
                            p = jnp.concatenate([w[:, j * 128:(j + 1) * 128] * xb for j in range(ncol)], axis=1)
                            p = p[0:8] + p[8:16]
                            acc = p if acc is None else acc + p
                        state["acc"] = acc
                        if k0 + rows == K:
                            moe[(key, c0)] = jnp.sum(acc, axis=0, keepdims=True)
                        return orall([bits(acc[:, j * 128:(j + 1) * 128]) for j in range(ncol)])
                    ts.append(task)
            return ts

        def hb_task(c0):
            def task(relbits):
                g = gate_all(st, jnp.broadcast_to(moe[("g", c0)], (8, MCOL * 128)), relbits)[0:1]
                u = moe[("u", c0)]
                g = rbf(g)
                h = rbf(rbf(g * (1.0 / (1.0 + jnp.exp(-g)))) * rbf(u))
                hb = jnp.broadcast_to(h, (128, MCOL * 128)).T
                hb_buf[pl.ds(c0 * 128, MCOL * 128), :] = hb
                return tile_bits_f32(hb)
            return task

        with scope(cfg, "stG"):
            nsub = (D // GN) * (S // GK)
            wqt = [wqT_task(j) for j in range(D // 128)]
            pre = [router_task(r) for r in range(0, S, RR)] + [router_final, zb_task] + (wqt if cfg.get("WQT_PRE", True) else [])
            post = []
            nhb_g = 0
            if MOE == "vpu":
                tg = mv_tasks(wg_buf, xb_buf, D, F // 128, "g", MCOL, MROWS)
                tu = mv_tasks(wu_buf, xb_buf, D, F // 128, "u", MCOL, MROWS)
                per = D // MROWS
                ngrp = len(tg) // per
                if cfg.get("POSTMIX", True):
                    HBLAG = cfg.get("HBLAG", 2)
                    hbq = []
                    for gi in range(ngrp):
                        for j, t in enumerate(tg[gi * per:(gi + 1) * per] + tu[gi * per:(gi + 1) * per]):
                            post.append(t)
                            if j == HBLAG - 1 and hbq:
                                post.append(hbq.pop(0)); nhb_g += 1
                        hbq.append(hb_task(gi * MCOL))
                else:
                    post = tg + tu
            if not cfg.get("WQT_PRE", True):
                post = wqt + post
            c_pre = spread(len(pre), 0, G1 - 1)
            c_post = spread(len(post), G1, nsub - cfg.get("GEND", 1))
            pi = qi = di = 0
            for n in range(D // GN):
                acc = None
                for kc in range(S // GK):
                    if di == G1:
                        wait(cfg.get("WG1", "wg wu"))
                    p = st.dot(pkT_buf[:, pl.ds(kc * GK, GK)], xn_buf[pl.ds(kc * GK, GK), pl.ds(n * GN, GN)], nk=NK)
                    acc = p if acc is None else acc + p
                    if kc == S // GK - 1:
                        g_buf[:, pl.ds(n * GN, GN)] = acc.astype(bf16)
                    for _ in range(c_pre.get(di, 0)):
                        PD = cfg.get("PREDL", DL)
                        st.side(pre[pi], rel=cfg.get("PREREL", REL), dl=PD if di + PD < G1 else None); pi += 1
                    for _ in range(c_post.get(di, 0)):
                        st.side(post[qi], rel=cfg.get("MREL", REL), dl=cfg.get("MDL", DL)); qi += 1
                    di += 1
            assert pi == len(pre) and qi == len(post)

        with scope(cfg, "stQ"):
            td = mv_tasks(wd_buf, hb_buf, F, D // 128, "d", DCOL, DROWS) if MOE == "vpu" else []
            rr = lax.broadcasted_iota(i32, (128, 128), 0) // DH
            cc = lax.broadcasted_iota(i32, (128, 128), 1) // DH
            bd = rr == cc

            def chain_task(c):
                def task(relbits):
                    kv = mm(g_buf[pl.ds(c * 128, 128), :], wv_buf[:, pl.ds(c * 128, 128)])
                    kv = jnp.where(bd, kv, 0.0).astype(bf16)
                    m_buf[pl.ds(c * 128, 128), :] = mm(kv, wo_buf[pl.ds(c * 128, 128), :]).astype(bf16)
                    return None
                return task

            kvs = {}

            def kv_task(c):
                def task(relbits):
                    kv = mm(g_buf[pl.ds(c * 128, 128), :], wv_buf[:, pl.ds(c * 128, 128)])
                    kvs[c] = jnp.where(bd, kv, 0.0).astype(bf16)
                    return None
                return task

            def m_task(c):
                def task(relbits):
                    m_buf[pl.ds(c * 128, 128), :] = mm(kvs[c], wo_buf[pl.ds(c * 128, 128), :]).astype(bf16)
                    return None
                return task

            def q_epilogue(t0, q):
                def task(relbits):
                    pq = phi(q)
                    zb = zb_buf[...]
                    tz = jnp.concatenate([pq[:, j * 128:(j + 1) * 128] * zb for j in range(QT // 128)], axis=1) if QT > 128 else pq * zb
                    den = jnp.sum(tz.reshape(H, DH, QT), axis=1, keepdims=True) + 1e-6
                    o = (pq.reshape(H, DH, QT) * (1.0 / den)).reshape(D, QT)
                    ot = o.astype(bf16).T
                    o_buf[pl.ds(t0, QT), :] = ot
                    return tile_bits_bf16(ot)
                return task

            nq = S // QT
            hbt = [hb_task(c0) for c0 in range(0, F // 128, MCOL)][nhb_g:] if MOE == "vpu" else []
            c_hb = spread(len(hbt), cfg.get("HB0", 0), max(cfg.get("HB0", 0) + 1, Q1 - 1))
            chain = [chain_task(c) for c in range(D // 128)]
            c_chain = spread(len(chain), Q1 + cfg.get("CH0", 0), min(nq, Q1 + cfg.get("CH0", 0) + cfg.get("CHN", 8)))
            CHS = cfg.get("CHSPLIT", 0)
            mq = {}
            c_down = spread(len(td), Q1, nq - cfg.get("DEND", 1))
            ci = dni = hi = 0
            deferred = None
            for qd in range(nq):
                t0 = qd * QT
                if qd == Q1:
                    wait("wv wo wd")
                    if MOE != "vpu":
                        x16 = jnp.broadcast_to(sel["xrow"], (16, D)).astype(bf16)
                        g = rbf(mm(x16, wg_buf[...]))
                        u = rbf(mm(x16, wu_buf[...]))
                        h = rbf(g * (1.0 / (1.0 + jnp.exp(-g)))) * u
                        ymx = mm(h.astype(bf16), wd_buf[...])[0:1, :]
                q = st.dot(wqT_buf[...], xn_buf[pl.ds(t0, QT), :], NT, nk=NK)
                if deferred is not None:
                    st.side(deferred, rel=None, dl=cfg.get("DEFDL", 2)); deferred = None
                ep = q_epilogue(t0, q)
                if qd + 1 == Q1 and cfg.get("DEFER", True):
                    deferred = ep
                else:
                    QE = cfg.get("QEDL", DL)
                    st.side(ep, rel=None, dl=QE if (not (qd < Q1 <= qd + QE) and qd + QE < nq + cfg.get("QTAIL", 2)) else None)
                for _ in range(c_hb.get(qd, 0)):
                    st.side(hbt[hi], rel=REL, dl=DL if qd + DL < Q1 else None); hi += 1
                for c in mq.pop(qd, []):
                    st.side(m_task(c), rel=None, dl=None)
                for _ in range(c_chain.get(qd, 0)):
                    if CHS:
                        st.side(kv_task(ci), rel=None, dl=None); mq.setdefault(min(qd + CHS, nq - 1), []).append(ci)
                    else:
                        st.side(chain[ci], rel=None, dl=None)
                    ci += 1
                for _ in range(c_down.get(qd, 0)):
                    st.side(td[dni], rel=cfg.get("DREL", REL), dl=cfg.get("DDL", DL) if qd + cfg.get("DDL", DL) <= nq else None); dni += 1
            assert ci == len(chain) and dni == len(td) and hi == len(hbt) and deferred is None and not mq
            if MOE == "vpu":
                y = jnp.concatenate([moe[("d", c0)] for c0 in range(0, D // 128, DCOL)], axis=1)
            else:
                y = ymx
            y = rbf(rbf(y) * sel["gate"])
            rows2 = jnp.where(sel["msk"], sel["rows"] + y, sel["rows"])
            xn_buf[pl.ds(sel["g0"], 16), :] = rows2.astype(bf16)

        with scope(cfg, "stD"):
            o_cp = []
            for n in range(NOUT):
                n0 = n * ON
                parts = DTAIL if n == NOUT - 1 else 1
                RB = S // parts
                for pp in range(parts):
                    r0 = pp * RB
                    acc = st.dot(o_buf[pl.ds(r0, RB), :], m_buf[:, pl.ds(n0, ON)], nk=NK, tie_row=min(cfg.get("DTIE", 1024), RB // 2))
                    res = xbuf[pl.ds(r0, RB), pl.ds(n0, ON)].astype(f32) + xn_buf[pl.ds(r0, RB), pl.ds(n0, ON)].astype(f32)
                    xbuf[pl.ds(r0, RB), pl.ds(n0, ON)] = (acc + res).astype(bf16)
                    c = pltpu.make_async_copy(xbuf.at[pl.ds(r0, RB), pl.ds(n0, ON)], out_hbm.at[pl.ds(r0, RB), pl.ds(n0, ON)], sems.at[cfg["OSEM"][len(o_cp) % len(cfg["OSEM"])]])
                    c.start()
                    o_cp.append(c)
            if cfg.get("ONEWAIT", True) and len(cfg["OSEM"]) == 1:
                pltpu.make_async_copy(xbuf, out_hbm, sems.at[cfg["OSEM"][0]]).wait()
            else:
                for c in o_cp:
                    c.wait()

    return kernel, len(XP) + 8 + len(cfg.get('QP', [0] * 4)), NOUT + DTAIL - 1


def _k_units(rows):
    return [(r0, 256, cb) for r0 in rows for cb in range(4)]


START_A = dict(
    XP=[256, 256, 256, 512, 768], ORDER="x0 x1 z q0 q1 x2 q2 q3 x3 wr x4 wq wg wu wv wo wd", W0="x0 x1 z", LN0=512,
    UNITS=[(0, 256, 0), (256, 256, 0), (0, 256, 1), (256, 256, 1), (0, 256, 2), (256, 256, 2), (512, 256, 0), (512, 256, 1), (512, 256, 2),
           (0, 256, 3), (256, 256, 3), (512, 256, 3)] + _k_units(range(768, 2048, 256)),
    WA={0: "q0", 2: "q1", 4: "q2 x2", 9: "q3 x3", 16: "x4 wr wq"},
    LNS=[(512, 768, 4, 6), (768, 1024, 9, 12), (1024, 1280, 10, 16), (1280, 1536, 16, 20), (1536, 1792, 18, 24), (1792, 2048, 22, 28)])
START_B = dict(
    XP=[256, 128, 128, 256, 512, 768], ORDER="q0 z x0 x1 x2 q1 q2 x3 q3 x4 wr x5 wq wg wu wv wo wd", W0="q0 z x0", LN0=256,
    UNITS=[(0, 256, 0), (256, 128, 0), (384, 128, 0), (0, 256, 1), (256, 256, 1), (0, 256, 2), (256, 256, 2), (512, 256, 0), (512, 256, 1), (512, 256, 2),
           (0, 256, 3), (256, 256, 3), (512, 256, 3)] + _k_units(range(768, 2048, 256)),
    WA={0: "x1", 1: "x2", 3: "q1", 5: "q2 x3", 10: "q3 x4", 17: "x5 wr wq"},
    LNS=[(256, 384, 0, 1), (384, 512, 1, 2), (512, 768, 5, 7), (768, 1024, 10, 13), (1024, 1280, 11, 17), (1280, 1536, 17, 21), (1536, 1792, 19, 25), (1792, 2048, 23, 29)])


def build(cfg=None):
    cfg = dict(cfg or {})
    for k, v in (START_B if cfg.get("START", "B") == "B" else START_A).items():
        cfg.setdefault(k, v)
    kernel, nin, nout = make_kernel(cfg)
    anyspec = pl.BlockSpec(memory_space=pl.ANY)
    scratch = [
        pltpu.VMEM((S, D), bf16),
        pltpu.VMEM((S, D), bf16),
        pltpu.VMEM((D, S), bf16),
        pltpu.VMEM((S, D), bf16),
        pltpu.VMEM((D, D), bf16),
        pltpu.VMEM((D, D), bf16),
        pltpu.VMEM((D, D), bf16),
        pltpu.VMEM((D, D), bf16),
        pltpu.VMEM((8, 128), bf16),
        pltpu.VMEM((D, F), bf16),
        pltpu.VMEM((D, F), bf16),
        pltpu.VMEM((F, D), bf16),
        pltpu.VMEM((D, D), bf16),
        pltpu.VMEM((D, D), bf16),
        pltpu.VMEM((D, D), bf16),
        pltpu.VMEM((D, 128), f32),
        pltpu.VMEM((D, 128), f32),
        pltpu.VMEM((F, 128), f32),
        pltpu.VMEM((16, 128), bf16),
        pltpu.SemaphoreType.DMA((max(list(cfg["SEM"].values()) + list(cfg["OSEM"])) + 1,)),
    ]
    call = pl.pallas_call(
        kernel,
        out_shape=jax.ShapeDtypeStruct((S, D), bf16),
        in_specs=[anyspec] * 7,
        out_specs=anyspec,
        scratch_shapes=scratch,
        compiler_params=pltpu.CompilerParams(vmem_limit_bytes=cfg.get("VMEM", 110) * 2**20, **cfg.get("CP", {})),
        interpret=cfg.get("INTERPRET", False),
    )

    def fn(A_x, A_wqkv, A_wo, B_x, B_w_r, B_w_gate, B_w_up, B_w_down):
        out = call(A_x.reshape(S, D), A_wqkv, A_wo, B_w_r.reshape(8, 128), B_w_gate, B_w_up, B_w_down)
        return out.reshape(1, S, D)

    return fn


_CFG = {'CHSPLIT': 2, 'CHN': 9, 'DROWS': 256, 'Q1': 2, 'POSTMIX': False, 'DREL': 2, 'PREREL': 3, 'MREL': 2, 'NK': 8, 'DDL': 3, 'PREDL': 4, 'LR': 32, 'XP': [256, 128, 128, 256, 512, 768], 'ORDER': 'x0 z x1 q0 x2 q1', 'W0': 'x0 z x1', 'LN0': 384, 'UNITS': [(0, 256, 0), (256, 128, 0), (384, 128, 0), (0, 256, 1), (256, 256, 1), (0, 256, 2), (256, 256, 2), (512, 128, 0), (512, 128, 1), (512, 128, 2), (640, 128, 0), (640, 128, 1), (640, 128, 2), (0, 256, 3), (256, 256, 3), (512, 256, 3), (768, 256, 0), (768, 256, 1), (768, 256, 2), (768, 256, 3), (1024, 256, 0), (1024, 256, 1), (1024, 256, 2), (1024, 256, 3), (1280, 256, 0), (1280, 256, 1), (1280, 256, 2), (1280, 256, 3), (1536, 256, 0), (1536, 256, 1), (1536, 256, 2), (1536, 256, 3), (1792, 256, 0), (1792, 256, 1), (1792, 256, 2), (1792, 256, 3)], 'WA': {0: 'q0', 1: 'x2', 3: 'q1', 5: 'q2 x3', 13: 'q3 x4', 20: 'x5 wr wq'}, 'LNS': [(384, 512, 1, 2), (512, 640, 5, 7), (640, 768, 7, 10), (768, 1024, 13, 16), (1024, 1280, 15, 19), (1280, 1536, 20, 24), (1536, 1792, 23, 27), (1792, 2048, 27, 31)], 'AFTER': {'x0 z x1': 'q2 x3', 'q0': 'q3 x4', 'x2': 'wr x5 wq', 'q2 x3': 'wg wu', 'q3 x4': 'wv wo wd'}, 'SEM': {'x0': 0, 'z': 0, 'x1': 0, 'q0': 1, 'x2': 2, 'q1': 3, 'q2': 0, 'x3': 0, 'q3': 1, 'x4': 1, 'wr': 2, 'x5': 2, 'wq': 2, 'wg': 0, 'wu': 0, 'wv': 1, 'wo': 1, 'wd': 1}, 'OSEM': [3], 'DTAIL': 8}


@jax.jit
def pallas_parallel_sum__linear_attn_block__moe_arch_mod__prompt_kernel(
    A_x: jax.Array,
    A_wqkv: jax.Array,
    A_wo: jax.Array,
    B_x: jax.Array,
    B_w_r: jax.Array,
    B_w_gate: jax.Array,
    B_w_up: jax.Array,
    B_w_down: jax.Array,
):
    return build(_CFG)(A_x, A_wqkv, A_wo, B_x, B_w_r, B_w_gate, B_w_up, B_w_down)
```

```python
import jax
import jax.numpy as jnp
import numpy as np
from jax import lax
from jax.experimental import pallas as pl
from jax.experimental.pallas import tpu as pltpu

S, D, F, H, DH = 2048, 1024, 3584, 32, 32
f32, bf16, i32, u32 = jnp.float32, jnp.bfloat16, jnp.int32, jnp.uint32

NN = (((1,), (0,)), ((), ()))
NT = (((1,), (1,)), ((), ()))
EPS_BF16 = np.float32(1.0013580322265625e-05)

X_ROWS = [256, 128, 128, 256, 512, 768]
DMA_FIRST = "x0 z x1 q0 x2 q1"
DMA_AFTER = {"x0 z x1": "q2 x3", "q0": "q3 x4", "x2": "wr x5 wq",
             "q2 x3": "wg wu", "q3 x4": "wv wo wd"}
DMA_SEM = dict(x0=0, z=0, x1=0, q0=1, x2=2, q1=3, q2=0, x3=0, q3=1, x4=1,
               wr=2, x5=2, wq=2, wg=0, wu=0, wv=1, wo=1, wd=1)
OUT_SEM = 3
N_SEM = 4

KN = 256
K_UNITS = ([(0, 256, 0), (256, 128, 0), (384, 128, 0), (0, 256, 1), (256, 256, 1), (0, 256, 2), (256, 256, 2),
            (512, 128, 0), (512, 128, 1), (512, 128, 2), (640, 128, 0), (640, 128, 1), (640, 128, 2),
            (0, 256, 3), (256, 256, 3), (512, 256, 3)]
           + [(r0, 256, cb) for r0 in range(768, S, 256) for cb in range(4)])
K_WAITS = {0: "q0", 1: "x2", 3: "q1", 5: "q2 x3", 13: "q3 x4", 20: "x5 wr wq"}
LN_FIRST = 384
LN_SLOTS = [(384, 512, 1, 2), (512, 640, 5, 7), (640, 768, 7, 10), (768, 1024, 13, 16),
            (1024, 1280, 15, 19), (1280, 1536, 20, 24), (1536, 1792, 23, 27), (1792, 2048, 27, 31)]
LR = 32
GK, GN = 512, 128
G1 = 11
RR = 64
MCOL, MROWS = 7, 256
DCOL, DROWS = 8, 256
QT = 128
Q1 = 2
ON = 128
D_TAIL = 8


def mm(a, b, dims=NN):
    return lax.dot_general(a, b, dims, preferred_element_type=f32)


def rbf(v):
    return v.astype(bf16).astype(f32)


def phi(t):
    return jnp.where(t > 0, t + 1.0, jnp.exp(t)) + 1e-6


def bits(v):
    return pltpu.bitcast(v, u32)


def orall(vs):
    f = vs[0]
    for o in vs[1:]:
        f = f | o
    return f


def tile_bits(v):
    rows = 16 if v.dtype == bf16 else 8
    return orall([bits(v[i * 128 + 128 - rows:(i + 1) * 128, j * 128:(j + 1) * 128])
                  for i in range(v.shape[0] // 128) for j in range(v.shape[1] // 128)])


def spread(ntasks, first, last):
    out, done = {}, 0
    for s in range(last - first):
        upto = ntasks * (s + 1) // (last - first)
        out[first + s] = upto - done
        done = upto
    return out


class Stream:
    def __init__(self):
        self.Z = None
        self.i = 0
        self.res = {}
        self.pend = {}

    def tie(self, target, src_bits):
        return pltpu.bitcast(pltpu.bitcast(target, u32) | (src_bits & self.Z), target.dtype)

    def dot(self, lhs, rhs, dims=NN, tie_row=0):
        fl = self.pend.pop(self.i, None)
        if fl:
            f = orall(fl)
            nk, r = min(8, lhs.shape[1] // 128), tie_row
            parts = [self.tie(lhs[r:r + 16, j * 128:(j + 1) * 128], f) for j in range(nk)]
            if nk * 128 < lhs.shape[1]:
                parts.append(lhs[r:r + 16, nk * 128:])
            top = jnp.concatenate(parts, axis=1)
            lhs = jnp.concatenate(([lhs[:r]] if r else []) + [top, lhs[r + 16:]], axis=0)
        p = mm(lhs, rhs, dims)
        self.res[self.i] = p[p.shape[0] - 8:, 0:128]
        self.i += 1
        return p

    def side(self, task, rel=1, dl=2):
        di = self.i - 1
        relv = self.res.get(di - rel) if rel is not None else None
        f = task(bits(relv) if relv is not None else None)
        if f is not None and dl is not None:
            self.pend.setdefault(di + dl, []).append(f)

    def gate(self, v, relbits, every=False):
        if relbits is None:
            return v
        if every:
            return jnp.concatenate([jnp.concatenate(
                [self.tie(v[i * 8:(i + 1) * 8, j * 128:(j + 1) * 128], relbits) for j in range(v.shape[1] // 128)], axis=1)
                for i in range(v.shape[0] // 8)], axis=0)
        row = self.tie(v[0:8, 0:128], relbits)
        if v.shape[1] > 128:
            row = jnp.concatenate([row, v[0:8, 128:]], axis=1)
        return row if v.shape[0] == 8 else jnp.concatenate([row, v[8:]], axis=0)


def _kernel(x_hbm, wqkv_hbm, wo_hbm, wr_hbm, wg_hbm, wu_hbm, wd_hbm, out_hbm,
            xbuf, xn_buf, pkT_buf, o_buf, wq_buf, wk_buf, wv_buf, wo_buf, wr_buf,
            wg_buf, wu_buf, wd_buf, wqT_buf, g_buf, m_buf, zb_buf, xb_buf, hb_buf, z2_buf, sems):
    def cp(nm, src, dst):
        return pltpu.make_async_copy(src, dst, sems.at[DMA_SEM[nm]])

    copies, r0 = {}, 0
    for i, n in enumerate(X_ROWS):
        copies["x%d" % i] = cp("x%d" % i, x_hbm.at[pl.ds(r0, n), :], xbuf.at[pl.ds(r0, n), :])
        r0 += n
    copies["z"] = cp("z", x_hbm.at[pl.ds(0, 16), pl.ds(0, 128)], z2_buf)
    copies["wr"] = cp("wr", wr_hbm, wr_buf)
    for j in range(4):
        copies["q%d" % j] = cp("q%d" % j, wqkv_hbm.at[:, pl.ds(D + j * KN, KN)], wk_buf.at[:, pl.ds(j * KN, KN)])
    copies["wq"] = cp("wq", wqkv_hbm.at[:, pl.ds(0, D)], wq_buf)
    copies["wv"] = cp("wv", wqkv_hbm.at[:, pl.ds(2 * D, D)], wv_buf)
    copies["wo"] = cp("wo", wo_hbm, wo_buf)
    copies["wg"] = cp("wg", wg_hbm, wg_buf)
    copies["wu"] = cp("wu", wu_hbm, wu_buf)
    copies["wd"] = cp("wd", wd_hbm, wd_buf)
    for nm in DMA_FIRST.split():
        copies[nm].start()

    st = Stream()

    def wait(lst):
        for nm in lst.split():
            copies[nm].wait()
        for nm in DMA_AFTER.get(lst, "").split():
            copies[nm].start()
        st.res = {}

    def ln_task(r0):
        def task(relbits):
            x = st.gate(xbuf[pl.ds(r0, LR), :].astype(f32), relbits)
            mean = jnp.sum(x, axis=1, keepdims=True) * (1.0 / D)
            d = x - mean
            var = jnp.sum(d * d, axis=1, keepdims=True) * (1.0 / D)
            std = rbf(jnp.sqrt(rbf(rbf(var) + EPS_BF16)))
            xn = d * (1.0 / std)
            xn_buf[pl.ds(r0, LR), :] = xn.astype(bf16)
            return orall([bits(xn[g * 8:(g + 1) * 8, D - 128:D]) for g in range(LR // 8)])
        return task

    zacc = {}
    wait("x0 z x1")
    for r in range(0, LN_FIRST, LR):
        ln_task(r)(None)
    st.Z = bits(z2_buf[...]) ^ bits(xbuf[0:16, 0:128])
    slots = {}
    for (a, b, u0, u1) in LN_SLOTS:
        tl = [ln_task(r) for r in range(a, b, LR)]
        u_need = min(ui for ui, (r0, nr, _) in enumerate(K_UNITS) if r0 < b and r0 + nr > a)
        cnt = spread(len(tl), u0, u1)
        for j in range(u0, u1):
            for _ in range(cnt[j]):
                slots.setdefault(j, []).append((tl.pop(0), u_need))

    def k_epilogue(r0, nr, cb, p):
        def task(relbits):
            pk = phi(p)
            zp = jnp.sum(pk.reshape(nr // 8, 8, KN), axis=0)
            zacc[cb] = zp if cb not in zacc else zacc[cb] + zp
            pt = pk.astype(bf16).T
            pkT_buf[pl.ds(cb * KN, KN), pl.ds(r0, nr)] = pt
            return tile_bits(pt)
        return task

    deferred = None
    for ui, (r0, nr, cb) in enumerate(K_UNITS):
        if ui in K_WAITS:
            wait(K_WAITS[ui])
        p = st.dot(xn_buf[pl.ds(r0, nr), :], wk_buf[:, pl.ds(cb * KN, KN)])
        nxtw = min([w for w in K_WAITS if w > ui] + [10 ** 9])
        if deferred is not None:
            st.side(deferred, rel=None, dl=1 if ui + 1 < nxtw else None)
            deferred = None
        ep = k_epilogue(r0, nr, cb, p)
        if ui + 1 == nxtw:
            deferred = ep
        else:
            st.side(ep, rel=None, dl=2 if ui + 2 < nxtw else None)
        for (t, u_need) in slots.get(ui, []):
            dl = min(2, u_need - ui)
            st.side(t, rel=1, dl=dl if ui + dl < nxtw else None)

    rs, sel = {}, {}

    def router_task(r0):
        def task(relbits):
            if "wr" not in rs:
                w8 = wr_buf[...].astype(f32)
                rs["wr"] = jnp.concatenate([w8[j:j + 1, :] for j in range(8)], axis=1)
                rs["best"] = jnp.full((RR, 1), -jnp.inf, f32)
                rs["bidx"] = jnp.zeros((RR, 1), f32)
                rs["iota"] = lax.broadcasted_iota(i32, (RR, 1), 0).astype(f32)
            pr = st.gate(xn_buf[pl.ds(r0, RR), :].astype(f32), relbits) * rs["wr"]
            sp = pr[:, 0:128]
            for j in range(1, D // 128):
                sp = sp + pr[:, j * 128:(j + 1) * 128]
            r = rbf(jnp.sum(sp, axis=1, keepdims=True))
            c = r > rs["best"]
            rs["best"] = jnp.where(c, r, rs["best"])
            rs["bidx"] = jnp.where(c, rs["iota"] + np.float32(r0), rs["bidx"])
            return orall([bits(sp[g * 8:(g + 1) * 8]) for g in range(RR // 8)])
        return task

    def router_final(relbits):
        best, bidx = rs["best"], rs["bidx"]
        cand = jnp.where(best == jnp.max(best), bidx, np.float32(2 * S))
        idx = jnp.clip(jnp.min(cand).astype(i32), 0, S - 1)
        g0 = pl.multiple_of((idx // 16) * 16, 16)
        rows = xn_buf[pl.ds(g0, 16), :].astype(f32)
        msk = lax.broadcasted_iota(i32, (16, D), 0) == (idx - g0)
        xrow = jnp.sum(jnp.where(msk, rows, 0.0), axis=0, keepdims=True)
        rsel = rbf(jnp.sum(xrow * rs["wr"], axis=1, keepdims=True))
        sel.update(g0=g0, rows=rows, msk=msk, gate=rbf(1.0 / (1.0 + jnp.exp(-rsel))))
        xb = jnp.broadcast_to(xrow, (128, D)).T
        xb_buf[...] = xb
        return tile_bits(xb)

    def zb_task(relbits):
        z = jnp.concatenate([jnp.sum(zacc[cb], axis=0, keepdims=True) for cb in range(D // KN)], axis=1)
        z = st.gate(jnp.broadcast_to(z, (8, D)), relbits)
        zb = jnp.broadcast_to(z[0:1], (128, D)).T
        zb_buf[...] = zb
        return tile_bits(zb)

    def wqT_task(j):
        def task(relbits):
            w = wq_buf[:, pl.ds(j * 128, 128)]
            if relbits is not None:
                w = jnp.concatenate([st.tie(w[0:16], relbits), w[16:]], axis=0)
            wt = w.T
            wqT_buf[pl.ds(j * 128, 128), :] = wt
            return tile_bits(wt)
        return task

    moe = {}

    def mv_tasks(w_ref, b_ref, K, ncolt, key, ncol, rows):
        ts = []
        for c0 in range(0, ncolt, ncol):
            state = {}
            for k0 in range(0, K, rows):
                def task(relbits, c0=c0, k0=k0, state=state):
                    acc = state.get("acc")
                    for k in range(k0, k0 + rows, 16):
                        w = w_ref[k:k + 16, c0 * 128:(c0 + ncol) * 128].astype(f32)
                        xb = b_ref[k:k + 16, :]
                        if k == k0:
                            xb = st.gate(xb, relbits)
                        p = jnp.concatenate([w[:, j * 128:(j + 1) * 128] * xb for j in range(ncol)], axis=1)
                        p = p[0:8] + p[8:16]
                        acc = p if acc is None else acc + p
                    state["acc"] = acc
                    if k0 + rows == K:
                        moe[(key, c0)] = jnp.sum(acc, axis=0, keepdims=True)
                    return orall([bits(acc[:, j * 128:(j + 1) * 128]) for j in range(ncol)])
                ts.append(task)
        return ts

    def hb_task(c0):
        def task(relbits):
            g = rbf(st.gate(jnp.broadcast_to(moe[("g", c0)], (8, MCOL * 128)), relbits, every=True)[0:1])
            h = rbf(rbf(g * (1.0 / (1.0 + jnp.exp(-g)))) * rbf(moe[("u", c0)]))
            hb = jnp.broadcast_to(h, (128, MCOL * 128)).T
            hb_buf[pl.ds(c0 * 128, MCOL * 128), :] = hb
            return tile_bits(hb)
        return task

    nsub = (D // GN) * (S // GK)
    pre = [router_task(r) for r in range(0, S, RR)] + [router_final, zb_task] + [wqT_task(j) for j in range(D // 128)]
    post = (mv_tasks(wg_buf, xb_buf, D, F // 128, "g", MCOL, MROWS)
            + mv_tasks(wu_buf, xb_buf, D, F // 128, "u", MCOL, MROWS))
    c_pre, c_post = spread(len(pre), 0, G1 - 1), spread(len(post), G1, nsub - 1)
    di = 0
    for n in range(D // GN):
        acc = None
        for kc in range(S // GK):
            if di == G1:
                wait("wg wu")
            p = st.dot(pkT_buf[:, pl.ds(kc * GK, GK)], xn_buf[pl.ds(kc * GK, GK), pl.ds(n * GN, GN)])
            acc = p if acc is None else acc + p
            if kc == S // GK - 1:
                g_buf[:, pl.ds(n * GN, GN)] = acc.astype(bf16)
            for _ in range(c_pre.get(di, 0)):
                st.side(pre.pop(0), rel=3, dl=4 if di + 4 < G1 else None)
            for _ in range(c_post.get(di, 0)):
                st.side(post.pop(0), rel=2, dl=2)
            di += 1

    down = mv_tasks(wd_buf, hb_buf, F, D // 128, "d", DCOL, DROWS)
    same_head = (lax.broadcasted_iota(i32, (128, 128), 0) // DH) == (lax.broadcasted_iota(i32, (128, 128), 1) // DH)
    kvs = {}

    def kv_task(c):
        kv = mm(g_buf[pl.ds(c * 128, 128), :], wv_buf[:, pl.ds(c * 128, 128)])
        kvs[c] = jnp.where(same_head, kv, 0.0).astype(bf16)

    def m_task(c):
        m_buf[pl.ds(c * 128, 128), :] = mm(kvs[c], wo_buf[pl.ds(c * 128, 128), :]).astype(bf16)

    def q_epilogue(t0, q):
        def task(relbits):
            pq = phi(q)
            den = jnp.sum((pq * zb_buf[...]).reshape(H, DH, QT), axis=1, keepdims=True) + 1e-6
            ot = (pq.reshape(H, DH, QT) * (1.0 / den)).reshape(D, QT).astype(bf16).T
            o_buf[pl.ds(t0, QT), :] = ot
            return tile_bits(ot)
        return task

    nq = S // QT
    hbt = [hb_task(c0) for c0 in range(0, F // 128, MCOL)]
    c_hb = spread(len(hbt), 0, max(1, Q1 - 1))
    c_kv = spread(D // 128, Q1, Q1 + 9)
    c_down = spread(len(down), Q1, nq - 1)
    m_at, ci, deferred = {}, 0, None
    for qd in range(nq):
        if qd == Q1:
            wait("wv wo wd")
        q = st.dot(wqT_buf[...], xn_buf[pl.ds(qd * QT, QT), :], NT)
        if deferred is not None:
            st.side(deferred, rel=None, dl=2)
            deferred = None
        ep = q_epilogue(qd * QT, q)
        if qd + 1 == Q1:
            deferred = ep
        else:
            st.side(ep, rel=None, dl=2 if (not (qd < Q1 <= qd + 2) and qd + 2 < nq + 2) else None)
        for _ in range(c_hb.get(qd, 0)):
            st.side(hbt.pop(0), rel=1, dl=2 if qd + 2 < Q1 else None)
        for c in m_at.pop(qd, []):
            m_task(c)
        for _ in range(c_kv.get(qd, 0)):
            kv_task(ci)
            m_at.setdefault(min(qd + 2, nq - 1), []).append(ci)
            ci += 1
        for _ in range(c_down.get(qd, 0)):
            st.side(down.pop(0), rel=2, dl=3 if qd + 3 <= nq else None)

    y = jnp.concatenate([moe[("d", c0)] for c0 in range(0, D // 128, DCOL)], axis=1)
    y = rbf(rbf(y) * sel["gate"])
    xn_buf[pl.ds(sel["g0"], 16), :] = jnp.where(sel["msk"], sel["rows"] + y, sel["rows"]).astype(bf16)

    for n0 in range(0, D, ON):
        parts = D_TAIL if n0 + ON == D else 1
        rb = S // parts
        for r0 in range(0, S, rb):
            acc = st.dot(o_buf[pl.ds(r0, rb), :], m_buf[:, pl.ds(n0, ON)], tie_row=min(1024, rb // 2))
            res = xbuf[pl.ds(r0, rb), pl.ds(n0, ON)].astype(f32) + xn_buf[pl.ds(r0, rb), pl.ds(n0, ON)].astype(f32)
            xbuf[pl.ds(r0, rb), pl.ds(n0, ON)] = (acc + res).astype(bf16)
            pltpu.make_async_copy(xbuf.at[pl.ds(r0, rb), pl.ds(n0, ON)], out_hbm.at[pl.ds(r0, rb), pl.ds(n0, ON)],
                                  sems.at[OUT_SEM]).start()
    pltpu.make_async_copy(xbuf, out_hbm, sems.at[OUT_SEM]).wait()


def _scratch():
    return [
        pltpu.VMEM((S, D), bf16),
        pltpu.VMEM((S, D), bf16),
        pltpu.VMEM((D, S), bf16),
        pltpu.VMEM((S, D), bf16),
        pltpu.VMEM((D, D), bf16),
        pltpu.VMEM((D, D), bf16),
        pltpu.VMEM((D, D), bf16),
        pltpu.VMEM((D, D), bf16),
        pltpu.VMEM((8, 128), bf16),
        pltpu.VMEM((D, F), bf16),
        pltpu.VMEM((D, F), bf16),
        pltpu.VMEM((F, D), bf16),
        pltpu.VMEM((D, D), bf16),
        pltpu.VMEM((D, D), bf16),
        pltpu.VMEM((D, D), bf16),
        pltpu.VMEM((D, 128), f32),
        pltpu.VMEM((D, 128), f32),
        pltpu.VMEM((F, 128), f32),
        pltpu.VMEM((16, 128), bf16),
        pltpu.SemaphoreType.DMA((N_SEM,)),
    ]


@jax.jit
def pallas_parallel_sum__linear_attn_block__moe_arch_mod__prompt_kernel(
    A_x: jax.Array,
    A_wqkv: jax.Array,
    A_wo: jax.Array,
    B_x: jax.Array,
    B_w_r: jax.Array,
    B_w_gate: jax.Array,
    B_w_up: jax.Array,
    B_w_down: jax.Array,
):
    del B_x
    anyspec = pl.BlockSpec(memory_space=pl.ANY)
    out = pl.pallas_call(
        _kernel,
        out_shape=jax.ShapeDtypeStruct((S, D), bf16),
        in_specs=[anyspec] * 7,
        out_specs=anyspec,
        scratch_shapes=_scratch(),
        compiler_params=pltpu.CompilerParams(vmem_limit_bytes=110 * 2**20),
    )(A_x.reshape(S, D), A_wqkv, A_wo, B_w_r.reshape(8, 128), B_w_gate, B_w_up, B_w_down)
    return out.reshape(1, S, D)
```
